```python
import os as _os
_os.environ.setdefault("JAX_PLATFORMS", "cpu")
import jax
import jax.numpy as jnp

def _softmax(x, axis=-1):
    return jax.nn.softmax(x, axis=axis)
def _gelu(x):
    return jax.nn.gelu(x, approximate=True)
def _silu(x):
    return jax.nn.silu(x)
def _sigmoid(x):
    return jax.nn.sigmoid(x)
def _layernorm(x, axis=-1, eps=1e-5):
    m = jnp.mean(x, axis=axis, keepdims=True)
    v = jnp.var(x, axis=axis, keepdims=True)
    return (x - m) / jnp.sqrt(v + eps)
def _scatter_add(tgt, idx, src, axis=0):
    return tgt.at[idx].add(src)
def _segment_sum(src, seg, n):
    return jax.ops.segment_sum(src, seg, n)
class _Rng:
    def __init__(self, key):
        self._k = key
    def _next(self):
        self._k, sub = jax.random.split(self._k)
        return sub
    def normal(self, shape):
        return jax.random.normal(self._next(), shape, dtype=jnp.bfloat16)
    def randint(self, lo, hi, shape):
        return jax.random.randint(self._next(), shape, lo, hi, dtype=jnp.int32)
    def uniform(self, shape, lo=0.0, hi=1.0):
        return jax.random.uniform(self._next(), shape, jnp.bfloat16, lo, hi)
    def permutation(self, n):
        return jax.random.permutation(self._next(), n)


kernel_name = 'concat_heads__mha_block_cached__gqa_block_cached__near_ridge'

def setup_inputs():
    _rng = _Rng(jax.random.key(int.from_bytes(__import__("os").urandom(4), "little")))
    _w = (lambda a: (lambda t: t.astype(jnp.bfloat16) if jnp.issubdtype(t.dtype, jnp.floating) else t)(jnp.asarray(a)))
    def _A_setup():
        B, Sq, D = 8, 128, 640
        H, Sk, Dh = 32, 1024, 192
        return {
            "x": _w((lambda *s: _rng.normal(s) * 0.8)(B, Sq, D)),
            "k_cache": _w((lambda *s: _rng.normal(s) * 0.8)(B, H, Sk, Dh)),
            "v_cache": _w((lambda *s: _rng.normal(s) * 0.05)(B, H, Sk, Dh)),
            "wq": _w((lambda *s: _rng.normal(s) * 0.8)(D, H * Dh) * (D ** -0.5)),
            "wo": _w((lambda *s: _rng.normal(s) * 0.05)(H * Dh, D) * ((H * Dh) ** -0.5)),
        }
    _A_in = _A_setup()

    def _B_setup():
        B, Sq, D = 8, 128, 640
        Hq, Hkv, Sk, Dh = 32, 32, 1024, 192
        assert Hq % Hkv == 0, (Hq, Hkv)
        return {
            "x": _w((lambda *s: _rng.normal(s) * 0.8)(B, Sq, D)),
            "k_cache": _w((lambda *s: _rng.normal(s) * 0.8)(B, Hkv, Sk, Dh)),
            "v_cache": _w((lambda *s: _rng.normal(s) * 0.05)(B, Hkv, Sk, Dh)),
            "wq": _w((lambda *s: _rng.normal(s) * 0.8)(D, Hq * Dh) * (D ** -0.5)),
            "wo": _w((lambda *s: _rng.normal(s) * 0.05)(Hq * Dh, D) * ((Hq * Dh) ** -0.5)),
        }
    _B_in = _B_setup()

    return {
        "A_x": _A_in["x"],
        "A_k_cache": _A_in["k_cache"],
        "A_v_cache": _A_in["v_cache"],
        "A_wq": _A_in["wq"],
        "A_wo": _A_in["wo"],
        "B_x": _B_in["x"],
        "B_k_cache": _B_in["k_cache"],
        "B_v_cache": _B_in["v_cache"],
        "B_wq": _B_in["wq"],
        "B_wo": _B_in["wo"],
    }

def reference(A_x, A_k_cache, A_v_cache, A_wq, A_wo, B_x, B_k_cache, B_v_cache, B_wq, B_wo):
    def _A_ref(x, k_cache, v_cache, wq, wo):
        B, Sq, D = x.shape
        H, Dh = 32, 192
        q = (lambda x, *d: x.transpose(*d))((x @ wq).reshape(B, Sq, H, Dh), 0, 2, 1, 3)
        scores = jnp.einsum("bhqd,bhkd->bhqk", q, k_cache) * (Dh ** -0.5)
        p = _softmax(scores, axis=-1)
        o = jnp.einsum("bhqk,bhkd->bhqd", p, v_cache)
        return (lambda x, *d: x.transpose(*d))(o, 0, 2, 1, 3).reshape(B, Sq, H * Dh) @ wo

    def _B_ref(x, k_cache, v_cache, wq, wo):
        B, Sq, D = x.shape
        Hq, Dh = 32, 192
        Hkv = k_cache.shape[1]
        rep = Hq // Hkv
        q = (lambda x, *d: x.transpose(*d))((x @ wq).reshape(B, Sq, Hq, Dh), 0, 2, 1, 3)
        k = jnp.repeat(k_cache, rep, axis=1)
        v = jnp.repeat(v_cache, rep, axis=1)
        scores = jnp.einsum("bhqd,bhkd->bhqk", q, k) * (Dh ** -0.5)
        p = _softmax(scores, axis=-1)
        o = jnp.einsum("bhqk,bhkd->bhqd", p, v)
        return (lambda x, *d: x.transpose(*d))(o, 0, 2, 1, 3).reshape(B, Sq, Hq * Dh) @ wo

    a = _A_ref(A_x, A_k_cache, A_v_cache, A_wq, A_wo)
    b = _B_ref(B_x, B_k_cache, B_v_cache, B_wq, B_wo)
    return jnp.concatenate([a, b], axis=-1)
```

```python
import functools
import math
import jax
import jax.numpy as jnp
from jax import lax
import jax.experimental.pallas as pl
import jax.experimental.pallas.tpu as pltpu

B, SQ, D = 8, 128, 640
H, SK, DH = 32, 1024, 192
F32 = jnp.float32
BF16 = jnp.bfloat16


def _kernel(xa, ka, va, wqa, woa, xb, kb, vb, wqb, wob, o_hbm,
            x_buf, kv_buf, wq_buf, wo_buf, acc_ref, o_buf,
            x_sem, kv_sem, w_sem, o_sem, *, HB, NBUF, nodma, nocompute):
    NHG = H // HB
    NS = NHG * B
    W = HB * DH
    NP = HB // 2
    scale = (DH ** -0.5) * math.log2(math.e)
    kv_srcs = (ka, kb, va, vb)

    def kv_copies(i, slot):
        hg = i // B
        b = i % B
        return [pltpu.make_async_copy(s.at[b, pl.ds(hg * HB, HB)], kv_buf.at[slot, j], kv_sem.at[slot, j])
                for j, s in enumerate(kv_srcs)]

    def w_copies(hg, slot):
        off = pl.multiple_of(hg * W, 128)
        return [
            pltpu.make_async_copy(wqa.at[:, pl.ds(off, W)], wq_buf.at[slot, 0], w_sem.at[slot, 0]),
            pltpu.make_async_copy(wqb.at[:, pl.ds(off, W)], wq_buf.at[slot, 1], w_sem.at[slot, 1]),
            pltpu.make_async_copy(woa.at[pl.ds(off, W), :], wo_buf.at[slot, 0], w_sem.at[slot, 2]),
            pltpu.make_async_copy(wob.at[pl.ds(off, W), :], wo_buf.at[slot, 1], w_sem.at[slot, 3]),
        ]

    def x_copies():
        return [pltpu.make_async_copy(xa, x_buf.at[0], x_sem.at[0]),
                pltpu.make_async_copy(xb, x_buf.at[1], x_sem.at[1])]

    def o_copy(b):
        return pltpu.make_async_copy(o_buf.at[b], o_hbm.at[b], o_sem.at[b])

    for c in x_copies(): c.start()
    for c in w_copies(0, 0): c.start()
    for i in range(NBUF - 1):
        for c in kv_copies(i, i): c.start()
    for c in x_copies(): c.wait()

    lane = lax.broadcasted_iota(jnp.int32, (SQ, 128), 1)
    ones = jnp.ones((16, SK), BF16)

    def body(i, carry):
        hg = i // B
        b = i % B
        slot = i % NBUF
        wslot = hg % 2
        nxt = i + NBUF - 1

        if not nodma:
            @pl.when(nxt < NS)
            def _():
                for c in kv_copies(nxt, nxt % NBUF): c.start()

        @pl.when(b == 0)
        def _():
            @pl.when(hg + 1 < NHG)
            def _():
                for c in w_copies(hg + 1, 1 - wslot): c.start()
            for c in w_copies(hg, wslot): c.wait()

        if nodma:
            @pl.when(i < NBUF - 1)
            def _():
                for c in kv_copies(i, slot): c.wait()
            slot = 0
        else:
            for c in kv_copies(i, slot): c.wait()

        @pl.when(hg == 0)
        def _():
            acc_ref[b] = jnp.zeros((SQ, 2 * D), F32)

        def qproj(pi):
            return jnp.dot(x_buf[pi, b], wq_buf[wslot, pi], preferred_element_type=F32) * scale

        def qk(pi, q, pr):
            kst = kv_buf[slot, pi, 2 * pr:2 * pr + 2].reshape(2 * DH, SK)
            qq = q[:, pr * 384:(pr + 1) * 384]
            q0 = qq[:, 0:128].astype(BF16)
            qm = qq[:, 128:256]
            q2 = qq[:, 256:384].astype(BF16)
            qlo = jnp.where(lane < 64, qm, 0.0).astype(BF16)
            qhi = jnp.where(lane >= 64, qm, 0.0).astype(BF16)
            qmid = jnp.concatenate([qlo, qhi], axis=0)
            d0 = jnp.dot(q0, kst[0:128], preferred_element_type=F32)
            dm = jnp.dot(qmid, kst[128:256], preferred_element_type=F32)
            d2 = jnp.dot(q2, kst[256:384], preferred_element_type=F32)
            return (d0 + dm[:SQ], dm[SQ:] + d2)

        def softmax(s):
            m = jnp.max(s, axis=-1, keepdims=True)
            return jnp.exp2(s - m).astype(BF16)

        def pv(pi, h, p):
            vt = jnp.concatenate([kv_buf[slot, 2 + pi, h], ones], axis=0)
            ot = lax.dot_general(vt, p, (((1,), (1,)), ((), ())), preferred_element_type=F32)
            return ot[:DH] * (1.0 / ot[DH:DH + 1])

        def oproj(pi, ots):
            o = jnp.concatenate(ots, axis=0).T.astype(BF16)
            contrib = jnp.dot(o, wo_buf[wslot, pi], preferred_element_type=F32)
            acc_ref[b, :, pi * D:(pi + 1) * D] += contrib

        if not nocompute:
            tasks = [(pi, pr) for pi in range(2) for pr in range(NP)]
            qs = {}
            ots = {0: [], 1: []}
            prev = None
            for (pi, pr) in tasks:
                if pi not in qs:
                    qs[pi] = qproj(pi)
                ss = qk(pi, qs[pi], pr)
                if prev is not None:
                    ppi, ppr, pps = prev
                    for j in range(2):
                        ots[ppi].append(pv(ppi, 2 * ppr + j, pps[j]))
                ps = [softmax(s) for s in ss]
                prev = (pi, pr, ps)
            ppi, ppr, pps = prev
            for j in range(2):
                ots[ppi].append(pv(ppi, 2 * ppr + j, pps[j]))
            oproj(0, ots[0])
            oproj(1, ots[1])

        @pl.when(hg == NHG - 1)
        def _():
            o_buf[b] = acc_ref[b].astype(BF16)
            o_copy(b).start()
        return carry

    lax.fori_loop(0, NS, body, 0)
    for b in range(B):
        o_copy(b).wait()


@jax.jit
def pallas_concat_heads__mha_block_cached__gqa_block_cached__near_ridge_kernel(
        A_x, A_k_cache, A_v_cache, A_wq, A_wo, B_x, B_k_cache, B_v_cache, B_wq, B_wo):
    HB, NBUF = 2, 3
    W = HB * DH
    t = lambda a: jnp.swapaxes(a, 2, 3)
    any_spec = pl.BlockSpec(memory_space=pl.ANY)
    return pl.pallas_call(
        functools.partial(_kernel, HB=HB, NBUF=NBUF, nodma=False, nocompute=False),
        in_specs=[any_spec] * 10,
        out_specs=any_spec,
        out_shape=jax.ShapeDtypeStruct((B, SQ, 2 * D), BF16),
        scratch_shapes=[
            pltpu.VMEM((2, B, SQ, D), BF16),
            pltpu.VMEM((NBUF, 4, HB, DH, SK), BF16),
            pltpu.VMEM((2, 2, D, W), BF16),
            pltpu.VMEM((2, 2, W, D), BF16),
            pltpu.VMEM((B, SQ, 2 * D), F32),
            pltpu.VMEM((B, SQ, 2 * D), BF16),
            pltpu.SemaphoreType.DMA((2,)),
            pltpu.SemaphoreType.DMA((NBUF, 4)),
            pltpu.SemaphoreType.DMA((2, 4)),
            pltpu.SemaphoreType.DMA((B,)),
        ],
        compiler_params=pltpu.CompilerParams(vmem_limit_bytes=64 * 1024 * 1024),
    )(A_x, t(A_k_cache), t(A_v_cache), A_wq, A_wo, B_x, t(B_k_cache), t(B_v_cache), B_wq, B_wo)
```

```python
import functools
import math
import jax
import jax.numpy as jnp
from jax import lax
import jax.experimental.pallas as pl
import jax.experimental.pallas.tpu as pltpu

B, SQ, D = 8, 128, 640
H, SK, DH = 32, 1024, 192
F32 = jnp.float32
BF16 = jnp.bfloat16
HB = 2
NHG = H // HB
NS = NHG * B
W = HB * DH
R = HB * DH


def mkseq(name, rows):
    per = R // rows
    if name == "rr":
        return [(j, t * rows, j % 2) for t in range(per) for j in range(4)]
    if name == "half":
        return [(j, (t + p * (per // 2)) * rows, p) for t in range(per // 2) for j in range(4) for p in (0, 1)]
    if name == "rr8":
        return [(j, (t + h * (per // 2)) * rows, j % 2) for t in range(per // 2) for h in (0, 1) for j in range(4)]
    raise ValueError(name)


def _kernel(xa, ka, va, wqa, woa, xb, kb, vb, wqb, wob, o_hbm,
            x_buf, kv_buf, wq_buf, wo_buf, acc_ref, o_buf,
            x_sem, kv_sem, w_sem, o_sem, *, NB, rows, seqname, batches, shift, wmode, nodma):
    scale = (DH ** -0.5) * math.log2(math.e)
    srcs = (ka, kb, va, vb)
    wq_srcs = (wqa, wqb)
    wo_srcs = (woa, wob)
    seq = mkseq(seqname, rows)
    n = len(seq)
    assert sum(batches) == n, (batches, n)
    issue = [(1, s) for s in seq[shift:]] + [(2, s) for s in seq[:shift]]

    def row0(i):
        hg = i // B
        b = i % B
        return pl.multiple_of((b * H + hg * HB) * DH, 64)

    def kv_rows(i, j, r0, m):
        slot = i % NB
        return pltpu.make_async_copy(srcs[j].at[pl.ds(row0(i) + r0, m)],
                                     kv_buf.at[slot, j, pl.ds(r0, m)], kv_sem.at[slot, j])

    def wq_rows(hg, pi, r0, m):
        off = pl.multiple_of(hg * W, 128)
        return pltpu.make_async_copy(wq_srcs[pi].at[pl.ds(r0, m), pl.ds(off, W)],
                                     wq_buf.at[hg % 2, pi, pl.ds(r0, m)], w_sem.at[hg % 2, pi])

    def wo_rows(hg, pi, r0, m):
        return pltpu.make_async_copy(wo_srcs[pi].at[pl.ds(pl.multiple_of(hg * W + r0, 8), m), :],
                                     wo_buf.at[hg % 2, pi, pl.ds(r0, m)], w_sem.at[hg % 2, 2 + pi])

    def w_full(hg):
        return [wq_rows(hg, 0, 0, D), wq_rows(hg, 1, 0, D), wo_rows(hg, 0, 0, W), wo_rows(hg, 1, 0, W)]

    def x_copies():
        return [pltpu.make_async_copy(xa, x_buf.at[0], x_sem.at[0]),
                pltpu.make_async_copy(xb, x_buf.at[1], x_sem.at[1])]

    def o_copy(b):
        return pltpu.make_async_copy(o_buf.at[b], o_hbm.at[b], o_sem.at[b])

    for c in x_copies(): c.start()
    for c in w_full(0): c.start()
    def pro(t, c):
        for j in range(4):
            kv_rows(0, j, pl.multiple_of(t * rows, 8), rows).start(priority=j % 2)
        return c
    lax.fori_loop(0, R // rows, pro, 0)
    acc_ref[...] = jnp.zeros(acc_ref.shape, F32)
    if not nodma:
        for (j, r0, p) in seq[:shift]: kv_rows(1, j, r0, rows).start(priority=p)
    for c in x_copies(): c.wait()
    if nodma:
        for j in range(4): kv_rows(0, j, 0, R).wait()

    lane = lax.broadcasted_iota(jnp.int32, (SQ, 128), 1)

    def body(i, carry, valid):
        hg = i // B
        b = i % B
        slot = 0 if nodma else i % NB
        wslot = hg % 2
        wvalid = hg + 1 < NHG
        st = dict(pos=0)

        def batch(k):
            lo = st["pos"]
            hi = lo + batches[k]
            st["pos"] = hi
            if nodma: return
            for (la, (j, r0, p)) in issue[lo:hi]:
                if valid[la]:
                    kv_rows(i + la, j, r0, rows).start(priority=p)

        def w_pieces(which):
            if wmode == "big": return
            @pl.when(wvalid)
            def _():
                for t in range(2):
                    for pi in range(2):
                        if which == "q":
                            wq_rows(hg + 1, pi, pl.multiple_of((b * 2 + t) * 40, 8), 40).start(priority=pi)
                        else:
                            wo_rows(hg + 1, pi, pl.multiple_of((b * 2 + t) * 24, 8), 24).start(priority=pi)

        batch(0)
        if wmode == "big":
            @pl.when((b == 0) & wvalid)
            def _():
                for c in w_full(hg + 1): c.start(priority=1)
        if not valid[1]:
            @pl.when(i == NS - 1)
            def _():
                for bb in range(B - 1):
                    o_copy(bb).start()
        @pl.when(b == 0)
        def _():
            for c in w_full(hg): c.wait()
        if not nodma:
            for j in range(4):
                kv_rows(i, j, 0, R).wait()

        def qproj(pi):
            return jnp.dot(x_buf[pi, b], wq_buf[wslot, pi], preferred_element_type=F32) * scale

        def qk(pi, q):
            q0 = q[:, 0:128].astype(BF16)
            qm = q[:, 128:256]
            q2 = q[:, 256:384].astype(BF16)
            qlo = jnp.where(lane < 64, qm, 0.0).astype(BF16)
            qhi = jnp.where(lane >= 64, qm, 0.0).astype(BF16)
            qs = (jnp.concatenate([q0, qlo], axis=1), jnp.concatenate([qhi, q2], axis=1))
            return [jnp.dot(qs[h], kv_buf[slot, pi, h * 128:h * 128 + 256, :], preferred_element_type=F32) for h in range(2)]

        def softmax(s):
            m = jnp.max(s, axis=-1, keepdims=True)
            p = jnp.exp2(s - m)
            return (p.astype(BF16), jnp.sum(p, axis=-1, keepdims=True))

        def pv(pi, h, pl_):
            p, l = pl_
            vt = kv_buf[slot, 2 + pi, h * DH:(h + 1) * DH, :]
            ot = lax.dot_general(vt, p, (((1,), (1,)), ((), ())), preferred_element_type=F32)
            return (ot, l)

        def oproj(pi, ots):
            o = jnp.concatenate([t[0] for t in ots], axis=0).T
            r0 = 1.0 / ots[0][1]
            r1 = 1.0 / ots[1][1]
            o = jnp.concatenate([o[:, 0:128] * r0, o[:, 128:256] * jnp.where(lane < 64, r0, r1), o[:, 256:384] * r1], axis=1)
            o = o.astype(BF16)
            acc_ref[b, :, pi * D:(pi + 1) * D] += jnp.dot(o, wo_buf[wslot, pi], preferred_element_type=F32)

        q0 = qproj(0)
        batch(1)
        s0 = qk(0, q0)
        w_pieces("q")
        q1 = qproj(1)
        batch(2)
        s1 = qk(1, q1)
        batch(3)
        p0 = [softmax(s) for s in s0]
        o0 = [pv(0, j, p0[j]) for j in range(2)]
        batch(4)
        p1 = [softmax(s) for s in s1]
        o1 = [pv(1, j, p1[j]) for j in range(2)]
        batch(5)
        oproj(0, o0)
        w_pieces("o")
        oproj(1, o1)

        @pl.when(hg == NHG - 1)
        def _():
            o_buf[b] = acc_ref[b].astype(BF16)
            @pl.when(b == B - 1)
            def _():
                o_copy(b).start()
        return carry

    lax.fori_loop(0, NS - 2, functools.partial(body, valid={1: True, 2: True}), 0)
    if shift < n:
        body(jnp.int32(NS - 2), 0, valid={1: True, 2: False})
        body(jnp.int32(NS - 1), 0, valid={1: False, 2: False})
    else:
        lax.fori_loop(NS - 2, NS, functools.partial(body, valid={1: False, 2: False}), 0)
    for b in range(B):
        o_copy(b).wait()


def build(NB=4, rows=16, seqname="rr", batches=(0, 16, 24, 16, 0, 40), shift=96, wmode="big", nodma=False):
    @jax.jit
    def f(A_x, A_k_cache, A_v_cache, A_wq, A_wo, B_x, B_k_cache, B_v_cache, B_wq, B_wo):
        t = lambda a: jnp.swapaxes(a, 2, 3).reshape(B * H * DH, SK)
        any_spec = pl.BlockSpec(memory_space=pl.ANY)
        return pl.pallas_call(
            functools.partial(_kernel, NB=NB, rows=rows, seqname=seqname, batches=batches, shift=shift, wmode=wmode, nodma=nodma),
            in_specs=[any_spec] * 10,
            out_specs=any_spec,
            out_shape=jax.ShapeDtypeStruct((B, SQ, 2 * D), BF16),
            scratch_shapes=[
                pltpu.VMEM((2, B, SQ, D), BF16),
                pltpu.VMEM((NB, 4, R, SK), BF16),
                pltpu.VMEM((2, 2, D, W), BF16),
                pltpu.VMEM((2, 2, W, D), BF16),
                pltpu.VMEM((B, SQ, 2 * D), F32),
                pltpu.VMEM((B, SQ, 2 * D), BF16),
                pltpu.SemaphoreType.DMA((2,)),
                pltpu.SemaphoreType.DMA((NB, 4)),
                pltpu.SemaphoreType.DMA((2, 4)),
                pltpu.SemaphoreType.DMA((B,)),
            ],
            compiler_params=pltpu.CompilerParams(vmem_limit_bytes=110 * 1024 * 1024, disable_bounds_checks=True),
        )(A_x, t(A_k_cache), t(A_v_cache), A_wq, A_wo, B_x, t(B_k_cache), t(B_v_cache), B_wq, B_wo)
    return f


pallas_concat_heads__mha_block_cached__gqa_block_cached__near_ridge_kernel = build(seqname="rr8")
```

```python
import functools
import math
import jax
import jax.numpy as jnp
from jax import lax
import jax.experimental.pallas as pl
import jax.experimental.pallas.tpu as pltpu

B, SQ, D = 8, 128, 640
H, SK, DH = 32, 1024, 192
F32 = jnp.float32
BF16 = jnp.bfloat16
HB = 2
NHG = H // HB
NS = NHG * B
W = HB * DH
R = HB * DH
NB = 4
NW = 4
NQ = 4
QH = 2
KV0 = 0
WQ0 = NB * 4 * R
WO0 = WQ0 + NW * D
TOT = WO0 + NW * 2 * W


def pieces(off):
    out = []
    rt, ct = divmod(off, 8)
    def clip(r0, nr, c0, nc):
        lo = max(r0, 0); hi = min(r0 + nr, R)
        return [(lo, hi - lo, c0, nc)] if hi > lo and nc > 0 else []
    for k in range(-1, R // 16):
        a = rt + 2 * k
        p = clip(a * 8, 16, ct * 128, SK - ct * 128) + clip((a + 1) * 8, 16, 0, ct * 128)
        if p: out.append(p)
    assert sum(nr * nc for p in out for (_, nr, _, nc) in p) == R * SK
    return out


def _kernel(xa, ka, va, wqa, woa, xb, kb, vb, wqb, wob, o_hbm,
            x_buf, big, q_buf, acc_ref, o_buf,
            x_sem, kv_sem, wq_sem, wo_sem, o_sem, *, off, stride, wts, LQ, LO, xrows, mode, order, shift):
    scale = (DH ** -0.5) * math.log2(math.e)
    srcs = (ka, kb, va, vb)
    wq_srcs = (wqa, wqb)
    wo_srcs = (woa, wob)
    x_srcs = (xa, xb)
    pcs = pieces(off)
    npc = len(pcs)
    assert math.gcd(stride, npc) == 1
    seq = [(j, pcs[(t * stride) % npc]) for t in range(npc) for j in range(4)]
    pairs = [seq[u:u + 2] for u in range(0, len(seq), 2)]
    sh = min(shift, len(pairs))
    sched = [(1, p) for p in pairs[sh:]] + [(2, p) for p in pairs[:sh]]
    cum = [0]
    for w_ in wts: cum.append(cum[-1] + w_)
    bounds = [round(c * len(pairs) / cum[-1]) for c in cum]

    def row0(i):
        hg = i // B
        b = i % B
        return pl.multiple_of((b * H + hg * HB) * DH, 64)

    def kv_base(i, j):
        return pl.multiple_of(KV0 + ((i % NB) * 4 + j) * R, 64)

    def kv_rect(i, j, r0, nr, c0, nc):
        return pltpu.make_async_copy(srcs[j].at[pl.ds(row0(i) + r0, nr), pl.ds(c0, nc)],
                                     big.at[pl.ds(kv_base(i, j) + r0, nr), pl.ds(c0, nc)], kv_sem.at[i % NB, j])

    def issue_pairs(i, prs):
        for pr in prs:
            for (j, p) in pr:
                for rc in p:
                    kv_rect(i, j, *rc).start(priority=j % 2)

    def wq_base(hg):
        return pl.multiple_of(WQ0 + (hg % NW) * D, 64)

    def wo_base(hg, pi):
        return pl.multiple_of(WO0 + ((hg % NW) * 2 + pi) * W, 64)

    def wq_rows(hg, pi, r0, m):
        offc = pl.multiple_of(hg * W, 128)
        return pltpu.make_async_copy(wq_srcs[pi].at[pl.ds(r0, m), pl.ds(offc, W)],
                                     big.at[pl.ds(pl.multiple_of(wq_base(hg) + r0, 8), m), pl.ds(pi * W, W)], wq_sem.at[hg % NW, pi])

    def wo_rows(hg, pi, r0, m):
        return pltpu.make_async_copy(wo_srcs[pi].at[pl.ds(pl.multiple_of(hg * W + r0, 8), m), :],
                                     big.at[pl.ds(pl.multiple_of(wo_base(hg, pi) + r0, 8), m), pl.ds(0, D)], wo_sem.at[hg % NW, pi])

    def wq_part(g):
        hg, part = g // B, g % B
        for t in range(2):
            for pi in range(2):
                wq_rows(hg, pi, pl.multiple_of((part * 2 + t) * 40, 8), 40).start(priority=pi)

    def wo_part(g):
        hg, part = g // B, g % B
        for t in range(2):
            for pi in range(2):
                wo_rows(hg, pi, pl.multiple_of((part * 2 + t) * 24, 8), 24).start(priority=pi)

    def x_rows(pi, r0, m):
        return pltpu.make_async_copy(x_srcs[pi].at[pl.ds(r0, m)], x_buf.at[pi, pl.ds(r0, m)], x_sem.at[pi])

    def o_copy(b):
        return pltpu.make_async_copy(o_buf.at[b], o_hbm.at[b], o_sem.at[b])

    lane = lax.broadcasted_iota(jnp.int32, (SQ, 128), 1)

    def qproj(i, pi):
        hg = i // B
        b = i % B
        x = x_buf[pi, pl.ds(pl.multiple_of(b * SQ, SQ), SQ), :]
        q = jnp.dot(x, big[pl.ds(wq_base(hg), D), pi * W:(pi + 1) * W], preferred_element_type=F32) * scale
        q0 = q[:, 0:128].astype(BF16)
        qm = q[:, 128:256]
        q2 = q[:, 256:384].astype(BF16)
        qlo = jnp.where(lane < 64, qm, 0.0).astype(BF16)
        qhi = jnp.where(lane >= 64, qm, 0.0).astype(BF16)
        q_buf[i % NQ, pi] = jnp.concatenate([q0, qlo, qhi, q2], axis=1)

    def loop(lo, hi, fn):
        def bd(t, c):
            fn(t)
            return c
        lax.fori_loop(lo, hi, bd, 0)

    loop(0, B * SQ // xrows, lambda t: [x_rows(pi, pl.multiple_of(t * xrows, 8), xrows).start(priority=pi) for pi in range(2)])
    loop(0, B, wq_part)
    acc_ref[...] = jnp.zeros(acc_ref.shape, F32)
    def pro(t):
        issue_pairs(t, pairs[:sh])
        if sh < len(pairs):
            @pl.when(t == 0)
            def _():
                issue_pairs(t, pairs[sh:])
        def wl(u):
            wo_part(t * (B // 2 + LO // 2) + u)
        loop(0, B // 2 + LO // 2, wl)
        loop(0, LQ // 2, lambda u: wq_part(B + t * (LQ // 2) + u))
        @pl.when(t == 0)
        def _():
            for pi in range(2):
                x_rows(pi, 0, B * SQ).wait()
            for pi in range(2):
                wq_rows(0, pi, 0, D).wait()
        for pi in range(2):
            qproj(t, pi)
    loop(0, 2, pro)

    def body(i, carry, issue, las):
        hg = i // B
        b = i % B
        st = dict(k=0)

        def tick():
            k = st["k"]
            st["k"] = k + 1
            for (la, p) in sched[bounds[k]:bounds[k + 1]]:
                if la in las:
                    issue_pairs(i + la, [p])

        def w_pieces(which):
            if not issue: return
            g = i + B + (LQ if which == "q" else LO)
            @pl.when(g < NS)
            def _():
                (wq_part if which == "q" else wo_part)(g)

        if not issue:
            @pl.when(i == NS - 1)
            def _():
                for bb in range(B - 1):
                    o_copy(bb).start()
        iq = i + QH
        if issue:
            @pl.when(iq % B == 0)
            def _():
                for pi in range(2):
                    wq_rows(iq // B, pi, 0, D).wait()
        @pl.when(b == 0)
        def _():
            for pi in range(2):
                wo_rows(hg, pi, 0, W).wait()
        for j in range(4):
            kv_rect(i, j, 0, R, 0, SK).wait()

        def putq(pi):
            tick()
            if issue:
                qproj(iq, pi)

        def qk(pi):
            q = q_buf[i % NQ, pi]
            out = []
            for h in range(2):
                tick()
                out.append(jnp.dot(q[:, h * 256:(h + 1) * 256], big[pl.ds(kv_base(i, pi) + h * 128, 256), :],
                                   preferred_element_type=F32))
            return out

        def softmax(s):
            m = jnp.max(s, axis=-1, keepdims=True)
            p = jnp.exp2(s - m)
            return (p.astype(BF16), jnp.sum(p, axis=-1, keepdims=True))

        def pv(pi, ps):
            out = []
            for h in range(2):
                tick()
                p, l = ps[h]
                vt = big[pl.ds(kv_base(i, 2 + pi) + h * DH, DH), :]
                out.append((lax.dot_general(vt, p, (((1,), (1,)), ((), ())), preferred_element_type=F32), l))
            return out

        def oproj(pi, ots):
            tick()
            o = jnp.concatenate([t[0] for t in ots], axis=0).T
            r0 = 1.0 / ots[0][1]
            r1 = 1.0 / ots[1][1]
            o = jnp.concatenate([o[:, 0:128] * r0, o[:, 128:256] * jnp.where(lane < 64, r0, r1), o[:, 256:384] * r1], axis=1)
            o = o.astype(BF16)
            acc_ref[b, :, pi * D:(pi + 1) * D] += jnp.dot(o, big[pl.ds(wo_base(hg, pi), W), 0:D], preferred_element_type=F32)

        if mode == "nocompute":
            for _ in range(13): tick()
            w_pieces("o"); w_pieces("q")
        else:
            s0 = qk(0)
            s1 = qk(1)
            p0 = [softmax(s) for s in s0]
            o0 = pv(0, p0)
            putq(0)
            p1 = [softmax(s) for s in s1]
            o1 = pv(1, p1)
            oproj(0, o0)
            w_pieces("q")
            putq(1)
            w_pieces("o")
            oproj(1, o1)
            tick()
        assert st["k"] == len(wts)

        @pl.when(hg == NHG - 1)
        def _():
            o_buf[b] = acc_ref[b].astype(BF16)
            @pl.when(b == B - 1)
            def _():
                o_copy(b).start()
        return carry

    lax.fori_loop(0, NS - 2, functools.partial(body, issue=True, las=(1, 2)), 0)
    if sh == len(pairs):
        lax.fori_loop(NS - 2, NS, functools.partial(body, issue=False, las=()), 0)
    else:
        body(jnp.int32(NS - 2), 0, issue=False, las=(1,))
        body(jnp.int32(NS - 1), 0, issue=False, las=())
    for b in range(B):
        o_copy(b).wait()


def build(off=13, stride=4, wts=(2, 4, 4, 4, 4, 0, 6, 4, 0, 6, 3, 3, 4), LQ=4, LO=2, xrows=32, mode="", order="late", shift=50):
    @jax.jit
    def f(A_x, A_k_cache, A_v_cache, A_wq, A_wo, B_x, B_k_cache, B_v_cache, B_wq, B_wo):
        t = lambda a: jnp.swapaxes(a, 2, 3).reshape(B * H * DH, SK)
        tx = lambda a: a.reshape(B * SQ, D)
        any_spec = pl.BlockSpec(memory_space=pl.ANY)
        return pl.pallas_call(
            functools.partial(_kernel, off=off, stride=stride, wts=wts, LQ=LQ, LO=LO, xrows=xrows, mode=mode, order=order, shift=shift),
            in_specs=[any_spec] * 10,
            out_specs=any_spec,
            out_shape=jax.ShapeDtypeStruct((B, SQ, 2 * D), BF16),
            scratch_shapes=[
                pltpu.VMEM((2, B * SQ, D), BF16),
                pltpu.VMEM((TOT, SK), BF16),
                pltpu.VMEM((NQ, 2, SQ, 512), BF16),
                pltpu.VMEM((B, SQ, 2 * D), F32),
                pltpu.VMEM((B, SQ, 2 * D), BF16),
                pltpu.SemaphoreType.DMA((2,)),
                pltpu.SemaphoreType.DMA((NB, 4)),
                pltpu.SemaphoreType.DMA((NW, 2)),
                pltpu.SemaphoreType.DMA((NW, 2)),
                pltpu.SemaphoreType.DMA((B,)),
            ],
            compiler_params=pltpu.CompilerParams(vmem_limit_bytes=110 * 1024 * 1024, disable_bounds_checks=True),
        )(tx(A_x), t(A_k_cache), t(A_v_cache), A_wq, A_wo, tx(B_x), t(B_k_cache), t(B_v_cache), B_wq, B_wo)
    return f


pallas_concat_heads__mha_block_cached__gqa_block_cached__near_ridge_kernel = build(shift=26, stride=21, wts=(0, 4, 4, 4, 4, 0, 6, 4, 0, 6, 3, 3, 6))
```

```python
import functools
import math
import jax
import jax.numpy as jnp
from jax import lax
import jax.experimental.pallas as pl
import jax.experimental.pallas.tpu as pltpu

B, SQ, D = 8, 128, 640
H, SK, DH = 32, 1024, 192
F32 = jnp.float32
BF16 = jnp.bfloat16
HB = 2
NHG = H // HB
NS = NHG * B
W = HB * DH
R = HB * DH
NB = 4
NW = 4
KV0 = 0
WQ0 = NB * 4 * R
WO0 = WQ0 + NW * D
TOT = WO0 + NW * 2 * W


def pieces(off):
    out = []
    rt, ct = divmod(off, 8)
    def clip(r0, nr, c0, nc):
        lo = max(r0, 0); hi = min(r0 + nr, R)
        return [(lo, hi - lo, c0, nc)] if hi > lo and nc > 0 else []
    for k in range(-1, R // 16):
        a = rt + 2 * k
        p = clip(a * 8, 16, ct * 128, SK - ct * 128) + clip((a + 1) * 8, 16, 0, ct * 128)
        if p: out.append(p)
    assert sum(nr * nc for p in out for (_, nr, _, nc) in p) == R * SK
    return out


def _kernel(xa, ka, va, wqa, woa, xb, kb, vb, wqb, wob, o_hbm,
            x_buf, big, q_buf, acc_ref, o_buf,
            x_sem, kv_sem, wq_sem, wo_sem, o_sem, *, off, stride, wts, twts, LW, xrows, shift, pre, scopes, mode, tl, nstat, wr):
    scale = (DH ** -0.5) * math.log2(math.e)
    srcs = (ka, kb, va, vb)
    wq_srcs = (wqa, wqb)
    wo_srcs = (woa, wob)
    x_srcs = (xa, xb)
    pcs = pieces(off)
    npc = len(pcs)
    assert math.gcd(stride, npc) == 1
    order = [(t * stride) % npc for t in range(npc)]
    H1N = (npc + 1) // 2

    def pre_cnt(s_):
        if s_ >= NS: return 0
        if s_ >= NS - len(tl): return tl[s_ - (NS - len(tl))]
        return H1N

    def frame(s_, generic=False):
        n0 = H1N if generic else (pre_cnt(s_) if s_ >= 0 else npc)
        n1 = H1N if generic else pre_cnt(s_ + 1)
        own, nxt = order[n0:], order[:n1]
        groups = []
        a = b_ = 0
        while a < len(own) or b_ < len(nxt):
            if b_ < len(nxt) and (a >= len(own) or b_ * len(own) <= a * len(nxt)):
                groups.append((1, nxt[b_])); b_ += 1
            else:
                groups.append((0, own[a])); a += 1
        return [(ds, [(j, pcs[k]), (j + 1, pcs[k])]) for (ds, k) in groups for j in (0, 2)]

    assert nstat >= len(tl) + 3
    sh = shift
    def sched_for(i_static):
        if i_static is None:
            f1 = f2 = frame(0, generic=True)
        else:
            f1 = frame(i_static + 1) if i_static + 1 < NS else []
            f2 = frame(i_static + 2) if i_static + 2 < NS else []
        return [(1 + ds, p) for (ds, p) in f1[sh:]] + [(2 + ds, p) for (ds, p) in f2[:sh]]
    OFFQ = 2 * B + LW
    OFFO = B + LW

    def mkbounds(ws, n_):
        cum = [0]
        for w_ in ws: cum.append(cum[-1] + w_)
        return [min(n_, round(c * max(n_, 40) / cum[-1])) for c in cum]

    import contextlib
    def scope(name):
        return jax.named_scope(name) if scopes else contextlib.nullcontext()

    def row0(i):
        hg = i // B
        b = i % B
        return pl.multiple_of((b * H + hg * HB) * DH, 64)

    def kv_base(i, j):
        return pl.multiple_of(KV0 + ((i % NB) * 4 + j) * R, 64)

    def kv_rect(i, j, r0, nr, c0, nc):
        return pltpu.make_async_copy(srcs[j].at[pl.ds(row0(i) + r0, nr), pl.ds(c0, nc)],
                                     big.at[pl.ds(kv_base(i, j) + r0, nr), pl.ds(c0, nc)], kv_sem.at[i % NB, j])

    def issue_pairs(i, prs):
        for pr in prs:
            for (j, p) in pr:
                for rc in p:
                    kv_rect(i, j, *rc).start(priority=j % 2)

    def wq_base(hg):
        return pl.multiple_of(WQ0 + (hg % NW) * D, 64)

    def wo_base(hg, pi):
        return pl.multiple_of(WO0 + ((hg % NW) * 2 + pi) * W, 64)

    def wq_rows(hg, pi, r0, m):
        offc = pl.multiple_of(hg * W, 128)
        return pltpu.make_async_copy(wq_srcs[pi].at[pl.ds(r0, m), pl.ds(offc, W)],
                                     big.at[pl.ds(pl.multiple_of(wq_base(hg) + r0, 8), m), pl.ds(pi * W, W)], wq_sem.at[hg % NW, pi])

    def wo_rows(hg, pi, r0, m):
        return pltpu.make_async_copy(wo_srcs[pi].at[pl.ds(pl.multiple_of(hg * W + r0, 8), m), :],
                                     big.at[pl.ds(pl.multiple_of(wo_base(hg, pi) + r0, 8), m), pl.ds(0, D)], wo_sem.at[hg % NW, pi])

    def wq_part(g):
        if "noq" in mode: return
        hg, part = g // B, g % B
        if "qA" in mode:
            for pi in range(2):
                wq_rows(hg, pi, pl.multiple_of(part * 80, 8), 80).start(priority=pi)
        elif "qB" in mode:
            for t in range(2):
                for pi in range(2):
                    u = part * 2 + t
                    base = (u // 4) * 20 + (u % 4)
                    for k in range(5):
                        wq_rows(hg, pi, pl.multiple_of((base + 4 * k) * 8, 8), 8).start(priority=pi)
        elif "qC" in mode:
            for t in range(2):
                for pi in range(2):
                    u = part * 2 + t
                    for k in range(5):
                        wq_rows(hg, pi, pl.multiple_of((u + 16 * k) * 8, 8), 8).start(priority=pi)
        elif "qD" in mode:
            for t in range(5):
                for pi in range(2):
                    wq_rows(hg, pi, pl.multiple_of((part * 5 + t) * 16, 8), 16).start(priority=pi)
        else:
            for t in range(2):
                for pi in range(2):
                    wq_rows(hg, pi, pl.multiple_of((part * 2 + t) * 40, 8), 40).start(priority=pi)

    def wo_part(g):
        if "noo" in mode: return
        hg, part = g // B, g % B
        for t in range(2):
            for pi in range(2):
                wo_rows(hg, pi, pl.multiple_of((part * 2 + t) * 24, 8), 24).start(priority=pi)

    def x_rows(pi, r0, m):
        return pltpu.make_async_copy(x_srcs[pi].at[pl.ds(r0, m)], x_buf.at[pi, pl.ds(r0, m)], x_sem.at[pi])

    def o_rect(r0, nr, c0, nc, k):
        return pltpu.make_async_copy(o_buf.at[pl.ds(r0, nr), pl.ds(c0, nc)], o_hbm.at[pl.ds(r0, nr), pl.ds(c0, nc)], o_sem.at[k])

    def o_first():
        m, ns, _ = wr
        n_ = (B - 1) * SQ // m
        h = -(-n_ // ns)
        for k in [k for t in range(h) for k in range(t, n_, h)]:
            o_rect(k * m, m, 0, 2 * D, 0).start()

    lane = lax.broadcasted_iota(jnp.int32, (SQ, 128), 1)

    def qproj(hg, b, pi):
        if "nc" in mode: return
        x = x_buf[pi, pl.ds(pl.multiple_of(b * SQ, SQ), SQ), :]
        q = jnp.dot(x, big[pl.ds(wq_base(hg), D), pi * W:(pi + 1) * W], preferred_element_type=F32) * scale
        q0 = q[:, 0:128].astype(BF16)
        qm = q[:, 128:256]
        q2 = q[:, 256:384].astype(BF16)
        qlo = jnp.where(lane < 64, qm, 0.0).astype(BF16)
        qhi = jnp.where(lane >= 64, qm, 0.0).astype(BF16)
        q_buf[b, pi] = jnp.concatenate([q0, qlo, qhi, q2], axis=1)

    def loop(lo, hi, fn):
        def bd(t, c):
            fn(t)
            return c
        lax.fori_loop(lo, hi, bd, 0)

    zero = jnp.int32(0) * pl.program_id(0) if False else 0
    if "nox" not in mode: loop(0, B * SQ // xrows, lambda t: [x_rows(pi, pl.multiple_of(t * xrows, 8), xrows).start(priority=pi) for pi in range(2)])
    loop(0, B, wq_part)
    acc_ref[...] = jnp.zeros(acc_ref.shape, F32)
    work = [functools.partial(issue_pairs, -1 + ds, [p]) for (ds, p) in frame(-1)]
    work += [functools.partial(issue_pairs, ds, [p]) for (ds, p) in frame(0)]
    work += [functools.partial(wo_part, g) for g in range(B)]
    work += [functools.partial(wq_part, g) for g in range(B, 2 * B)]
    work += [functools.partial(issue_pairs, 1 + ds, [p]) for (ds, p) in frame(1)[:sh]]
    work += [functools.partial(wo_part, g) for g in range(B, OFFO)]
    work += [functools.partial(wq_part, g) for g in range(2 * B, OFFQ)]
    for w_ in work[:pre]: w_()
    for pi in range(2):
        if "nox" not in mode: x_rows(pi, 0, B * SQ).wait()
    for pi in range(2):
        if "noq" not in mode: wq_rows(0, pi, 0, D).wait()
    rest = work[pre:]
    with scope("s_pro"):
        nq = 2 * B
        for u in range(nq):
            for w_ in rest[(u * len(rest)) // nq:((u + 1) * len(rest)) // nq]: w_()
            qproj(0, u // 2, u % 2)

    def body(i, carry, main, static):
        sched = sched_for(i if static else None)
        last = static and i == NS - 1
        hg = i // B
        b = i % B
        st = dict(k=0)
        bounds = mkbounds(wts if main else twts, len(sched))

        def tick():
            k = st["k"]
            st["k"] = k + 1
            for (la, p) in sched[bounds[k]:bounds[k + 1]]:
                issue_pairs(i + la, [p])

        def w_pieces():
            if not main: return
            @pl.when(i + OFFQ < NS)
            def _():
                wq_part(i + OFFQ)
            if LW == 0:
                wo_part(i + OFFO)
            else:
                @pl.when(i + OFFO < NS)
                def _():
                    wo_part(i + OFFO)

        if last:
            if "nc" not in mode: o_first()
        if not static or b == 0:
            @pl.when(b == 0)
            def _():
                if main and "noq" not in mode:
                    for pi in range(2):
                        wq_rows(hg + 1, pi, 0, D).wait()
                for pi in range(2):
                    if "noo" not in mode: wo_rows(hg, pi, 0, W).wait()
        with scope("w_%s" % (i if static else ("m" if main else "t"))):
            for j in range(4):
                kv_rect(i, j, 0, R, 0, SK).wait()

        def putq(pi):
            tick()
            if main:
                qproj(hg + 1, b, pi)

        def qk(pi):
            q = q_buf[b, pi]
            out = []
            for h in range(2):
                tick()
                out.append(jnp.dot(q[:, h * 256:(h + 1) * 256], big[pl.ds(kv_base(i, pi) + h * 128, 256), :],
                                   preferred_element_type=F32))
            return out

        def softmax(s):
            m = jnp.max(s, axis=-1, keepdims=True)
            p = jnp.exp2(s - m)
            return (p.astype(BF16), jnp.sum(p, axis=-1, keepdims=True))

        def pv(pi, ps):
            out = []
            for h in range(2):
                tick()
                p, l = ps[h]
                vt = big[pl.ds(kv_base(i, 2 + pi) + h * DH, DH), :]
                out.append((lax.dot_general(vt, p, (((1,), (1,)), ((), ())), preferred_element_type=F32), l))
            return out

        def oproj(pi, ots):
            tick()
            o = jnp.concatenate([t[0] for t in ots], axis=0).T
            r0 = 1.0 / ots[0][1]
            r1 = 1.0 / ots[1][1]
            o = jnp.concatenate([o[:, 0:128] * r0, o[:, 128:256] * jnp.where(lane < 64, r0, r1), o[:, 256:384] * r1], axis=1)
            o = o.astype(BF16)
            res = acc_ref[b, :, pi * D:(pi + 1) * D] + jnp.dot(o, big[pl.ds(wo_base(hg, pi), W), 0:D], preferred_element_type=F32)
            if main:
                acc_ref[b, :, pi * D:(pi + 1) * D] = res
            else:
                o_buf[pl.ds(pl.multiple_of(b * SQ, SQ), SQ), pi * D:(pi + 1) * D] = res.astype(BF16)
                if last and wr[2]:
                    o_rect((B - 1) * SQ, SQ, pi * D, D, 1).start()

        if "nc" in mode:
            tick(); tick(); w_pieces()
            for _ in range(11): tick()
            if last:
                o_buf[pl.ds((B - 1) * SQ, SQ), :] = acc_ref[B - 1].astype(BF16)
                o_rect((B - 1) * SQ, SQ, 0, 2 * D, 1).start()
            return carry
        s0 = qk(0)
        w_pieces()
        s1 = qk(1)
        p0 = [softmax(s) for s in s0]
        o0 = pv(0, p0)
        putq(0)
        p1 = [softmax(s) for s in s1]
        o1 = pv(1, p1)
        oproj(0, o0)
        putq(1)
        oproj(1, o1)
        tick()
        assert st["k"] == 13
        if last and not wr[2]:
            o_rect((B - 1) * SQ, SQ, 0, 2 * D, 1).start()
        return carry

    with scope("s_main"):
        lax.fori_loop(0, NS - B, functools.partial(body, main=True, static=False), 0)
    if nstat < B:
        with scope("s_tail"):
            lax.fori_loop(NS - B, NS - nstat, functools.partial(body, main=False, static=False), 0)
    for u in range(NS - nstat, NS):
        with scope("s_%d" % u):
            body(u, 0, main=False, static=True)
    with scope("s_fin"):
        if "nc" not in mode: o_rect(0, (B - 1) * SQ, 0, 2 * D, 0).wait()
        o_rect((B - 1) * SQ, SQ, 0, 2 * D, 1).wait()


def build(off=13, stride=1, wts=(0, 4, 3, 4, 4, 0, 6, 4, 0, 6, 4, 4, 6), twts=(0, 4, 4, 4, 4, 0, 0, 6, 0, 6, 0, 4, 6),
          LW=0, xrows=32, shift=26, pre=16, scopes=False, mode='', tl=(8, 4), nstat=5, wr=(32, 4, True)):
    @jax.jit
    def f(A_x, A_k_cache, A_v_cache, A_wq, A_wo, B_x, B_k_cache, B_v_cache, B_wq, B_wo):
        t = lambda a: jnp.swapaxes(a, 2, 3).reshape(B * H * DH, SK)
        tx = lambda a: a.reshape(B * SQ, D)
        any_spec = pl.BlockSpec(memory_space=pl.ANY)
        return pl.pallas_call(
            functools.partial(_kernel, off=off, stride=stride, wts=wts, twts=twts, LW=LW, xrows=xrows, shift=shift, pre=pre, scopes=scopes, mode=mode, tl=tl, nstat=nstat, wr=wr),
            in_specs=[any_spec] * 10,
            out_specs=any_spec,
            out_shape=jax.ShapeDtypeStruct((B * SQ, 2 * D), BF16),
            scratch_shapes=[
                pltpu.VMEM((2, B * SQ, D), BF16),
                pltpu.VMEM((TOT, SK), BF16),
                pltpu.VMEM((B, 2, SQ, 512), BF16),
                pltpu.VMEM((B, SQ, 2 * D), F32),
                pltpu.VMEM((B * SQ, 2 * D), BF16),
                pltpu.SemaphoreType.DMA((2,)),
                pltpu.SemaphoreType.DMA((NB, 4)),
                pltpu.SemaphoreType.DMA((NW, 2)),
                pltpu.SemaphoreType.DMA((NW, 2)),
                pltpu.SemaphoreType.DMA((2,)),
            ],
            compiler_params=pltpu.CompilerParams(vmem_limit_bytes=110 * 1024 * 1024, disable_bounds_checks=True),
        )(tx(A_x), t(A_k_cache), t(A_v_cache), A_wq, A_wo, tx(B_x), t(B_k_cache), t(B_v_cache), B_wq, B_wo).reshape(B, SQ, 2 * D)
    return f


pallas_concat_heads__mha_block_cached__gqa_block_cached__near_ridge_kernel = build(shift=28, stride=21, tl=(8,4,0), nstat=6, wr=(16,4,True))
```

```python
import functools
import math

import jax
import jax.numpy as jnp
from jax import lax
import jax.experimental.pallas as pl
import jax.experimental.pallas.tpu as pltpu

B, SQ, D = 8, 128, 640
H, SK, DH = 32, 1024, 192
F32 = jnp.float32
BF16 = jnp.bfloat16

HB = 2
NHG = H // HB
NS = NHG * B
W = HB * DH
R = HB * DH
NB = 4
NW = 4

WQ0 = NB * 4 * R
WO0 = WQ0 + NW * D
TOT = WO0 + NW * 2 * W

OFF = 13
STRIDE = 21
SHIFT = 28
TAIL_PRE = (8, 4, 0)
NSTAT = 6
PRE = 16
WTS = (0, 4, 3, 4, 4, 0, 6, 4, 0, 6, 4, 4, 6)
TWTS = (0, 4, 4, 4, 4, 0, 0, 6, 0, 6, 0, 4, 6)
XROWS = 32
OROWS, OSTREAMS = 16, 4


def _pieces():
    out = []
    rt, ct = divmod(OFF, 8)

    def clip(r0, nr, c0, nc):
        lo, hi = max(r0, 0), min(r0 + nr, R)
        return [(lo, hi - lo, c0, nc)] if hi > lo and nc > 0 else []

    for k in range(-1, R // 16):
        a = rt + 2 * k
        p = clip(a * 8, 16, ct * 128, SK - ct * 128) + clip((a + 1) * 8, 16, 0, ct * 128)
        if p:
            out.append(p)
    assert sum(nr * nc for p in out for (_, nr, _, nc) in p) == R * SK
    return out


_PCS = _pieces()
_NPC = len(_PCS)
assert math.gcd(STRIDE, _NPC) == 1
_ORDER = [(t * STRIDE) % _NPC for t in range(_NPC)]
_H1N = (_NPC + 1) // 2


def _pre_cnt(s):
    if s >= NS:
        return 0
    if s >= NS - len(TAIL_PRE):
        return TAIL_PRE[s - (NS - len(TAIL_PRE))]
    return _H1N


def _frame(s, generic=False):
    n0 = _H1N if generic else (_pre_cnt(s) if s >= 0 else _NPC)
    n1 = _H1N if generic else _pre_cnt(s + 1)
    own, nxt = _ORDER[n0:], _ORDER[:n1]
    groups, a, b = [], 0, 0
    while a < len(own) or b < len(nxt):
        if b < len(nxt) and (a >= len(own) or b * len(own) <= a * len(nxt)):
            groups.append((1, nxt[b]))
            b += 1
        else:
            groups.append((0, own[a]))
            a += 1
    return [(ds, [(j, _PCS[k]), (j + 1, _PCS[k])]) for (ds, k) in groups for j in (0, 2)]


def _sched(i_static):
    if i_static is None:
        f1 = f2 = _frame(0, generic=True)
    else:
        f1 = _frame(i_static + 1) if i_static + 1 < NS else []
        f2 = _frame(i_static + 2) if i_static + 2 < NS else []
    return [(1 + ds, p) for (ds, p) in f1[SHIFT:]] + [(2 + ds, p) for (ds, p) in f2[:SHIFT]]


def _bounds(ws, n):
    cum = [0]
    for w in ws:
        cum.append(cum[-1] + w)
    return [min(n, round(c * max(n, 40) / cum[-1])) for c in cum]


def _kernel(xa, ka, va, wqa, woa, xb, kb, vb, wqb, wob, o_hbm,
            x_buf, big, q_buf, acc_ref, o_buf,
            x_sem, kv_sem, wq_sem, wo_sem, o_sem):
    scale = (DH ** -0.5) * math.log2(math.e)
    kv_srcs = (ka, kb, va, vb)
    wq_srcs = (wqa, wqb)
    wo_srcs = (woa, wob)
    x_srcs = (xa, xb)

    def kv_base(i, j):
        return pl.multiple_of(((i % NB) * 4 + j) * R, 64)

    def kv_rect(i, j, r0, nr, c0, nc):
        row0 = pl.multiple_of(((i % B) * H + (i // B) * HB) * DH, 64)
        return pltpu.make_async_copy(
            kv_srcs[j].at[pl.ds(row0 + r0, nr), pl.ds(c0, nc)],
            big.at[pl.ds(kv_base(i, j) + r0, nr), pl.ds(c0, nc)],
            kv_sem.at[i % NB, j])

    def kv_pair(i, pair):
        for (j, piece) in pair:
            for rc in piece:
                kv_rect(i, j, *rc).start(priority=j % 2)

    def wq_base(hg):
        return pl.multiple_of(WQ0 + (hg % NW) * D, 64)

    def wo_base(hg, pi):
        return pl.multiple_of(WO0 + ((hg % NW) * 2 + pi) * W, 64)

    def wq_rows(hg, pi, r0, m):
        return pltpu.make_async_copy(
            wq_srcs[pi].at[pl.ds(r0, m), pl.ds(pl.multiple_of(hg * W, 128), W)],
            big.at[pl.ds(pl.multiple_of(wq_base(hg) + r0, 8), m), pl.ds(pi * W, W)],
            wq_sem.at[hg % NW, pi])

    def wo_rows(hg, pi, r0, m):
        return pltpu.make_async_copy(
            wo_srcs[pi].at[pl.ds(pl.multiple_of(hg * W + r0, 8), m), :],
            big.at[pl.ds(pl.multiple_of(wo_base(hg, pi) + r0, 8), m), pl.ds(0, D)],
            wo_sem.at[hg % NW, pi])

    def wq_part(g):
        m = D // (2 * B)
        for t in range(2):
            for pi in range(2):
                wq_rows(g // B, pi, pl.multiple_of(((g % B) * 2 + t) * m, 8), m).start(priority=pi)

    def wo_part(g):
        m = W // (2 * B)
        for t in range(2):
            for pi in range(2):
                wo_rows(g // B, pi, pl.multiple_of(((g % B) * 2 + t) * m, 8), m).start(priority=pi)

    def x_rows(pi, r0, m):
        return pltpu.make_async_copy(x_srcs[pi].at[pl.ds(r0, m)], x_buf.at[pi, pl.ds(r0, m)], x_sem.at[pi])

    def o_rect(r0, nr, c0, nc, k):
        return pltpu.make_async_copy(o_buf.at[pl.ds(r0, nr), pl.ds(c0, nc)],
                                     o_hbm.at[pl.ds(r0, nr), pl.ds(c0, nc)], o_sem.at[k])

    def loop(lo, hi, fn):
        def bd(t, c):
            fn(t)
            return c
        lax.fori_loop(lo, hi, bd, 0)

    lane = lax.broadcasted_iota(jnp.int32, (SQ, 128), 1)

    def qproj(hg, b, pi):
        x = x_buf[pi, pl.ds(pl.multiple_of(b * SQ, SQ), SQ), :]
        q = jnp.dot(x, big[pl.ds(wq_base(hg), D), pi * W:(pi + 1) * W],
                    preferred_element_type=F32) * scale
        qm = q[:, 128:256]
        q_buf[b, pi] = jnp.concatenate(
            [q[:, 0:128].astype(BF16),
             jnp.where(lane < 64, qm, 0.0).astype(BF16),
             jnp.where(lane >= 64, qm, 0.0).astype(BF16),
             q[:, 256:384].astype(BF16)], axis=1)

    def x_start(t):
        for pi in range(2):
            x_rows(pi, pl.multiple_of(t * XROWS, 8), XROWS).start(priority=pi)

    loop(0, B * SQ // XROWS, x_start)
    loop(0, B, wq_part)
    acc_ref[...] = jnp.zeros(acc_ref.shape, F32)
    work = [functools.partial(kv_pair, ds - 1, p) for (ds, p) in _frame(-1)]
    work += [functools.partial(kv_pair, ds, p) for (ds, p) in _frame(0)]
    work += [functools.partial(wo_part, g) for g in range(B)]
    work += [functools.partial(wq_part, g) for g in range(B, 2 * B)]
    work += [functools.partial(kv_pair, ds + 1, p) for (ds, p) in _frame(1)[:SHIFT]]
    for w in work[:PRE]:
        w()
    for pi in range(2):
        x_rows(pi, 0, B * SQ).wait()
    for pi in range(2):
        wq_rows(0, pi, 0, D).wait()
    rest = work[PRE:]
    for u in range(2 * B):
        for w in rest[(u * len(rest)) // (2 * B):((u + 1) * len(rest)) // (2 * B)]:
            w()
        qproj(0, u // 2, u % 2)

    def step(i, carry, main, static):
        hg = i // B
        b = i % B
        last = static and i == NS - 1
        sched = _sched(i if static else None)
        bounds = _bounds(WTS if main else TWTS, len(sched))
        pos = [0]

        def tick():
            k = pos[0]
            pos[0] = k + 1
            for (la, p) in sched[bounds[k]:bounds[k + 1]]:
                kv_pair(i + la, p)

        if last:
            n = (B - 1) * SQ // OROWS
            h = -(-n // OSTREAMS)
            for k in [k for t in range(h) for k in range(t, n, h)]:
                o_rect(k * OROWS, OROWS, 0, 2 * D, 0).start()
        if not static:
            @pl.when(b == 0)
            def _():
                if main:
                    for pi in range(2):
                        wq_rows(hg + 1, pi, 0, D).wait()
                for pi in range(2):
                    wo_rows(hg, pi, 0, W).wait()
        for j in range(4):
            kv_rect(i, j, 0, R, 0, SK).wait()

        def next_q(pi):
            tick()
            if main:
                qproj(hg + 1, b, pi)

        def scores(pi):
            q = q_buf[b, pi]
            out = []
            for h in range(2):
                tick()
                out.append(jnp.dot(q[:, h * 256:(h + 1) * 256],
                                   big[pl.ds(kv_base(i, pi) + h * 128, 256), :],
                                   preferred_element_type=F32))
            return out

        def softmax(s):
            m = jnp.max(s, axis=-1, keepdims=True)
            p = jnp.exp2(s - m)
            return p.astype(BF16), jnp.sum(p, axis=-1, keepdims=True)

        def values(pi, ps):
            out = []
            for h in range(2):
                tick()
                p, l = ps[h]
                vt = big[pl.ds(kv_base(i, 2 + pi) + h * DH, DH), :]
                out.append((lax.dot_general(vt, p, (((1,), (1,)), ((), ())),
                                            preferred_element_type=F32), l))
            return out

        def oproj(pi, ots):
            tick()
            o = jnp.concatenate([t[0] for t in ots], axis=0).T
            r0 = 1.0 / ots[0][1]
            r1 = 1.0 / ots[1][1]
            o = jnp.concatenate([o[:, 0:128] * r0,
                                 o[:, 128:256] * jnp.where(lane < 64, r0, r1),
                                 o[:, 256:384] * r1], axis=1).astype(BF16)
            res = acc_ref[b, :, pi * D:(pi + 1) * D] + jnp.dot(
                o, big[pl.ds(wo_base(hg, pi), W), 0:D], preferred_element_type=F32)
            if main:
                acc_ref[b, :, pi * D:(pi + 1) * D] = res
            else:
                o_buf[pl.ds(pl.multiple_of(b * SQ, SQ), SQ), pi * D:(pi + 1) * D] = res.astype(BF16)
                if last:
                    o_rect((B - 1) * SQ, SQ, pi * D, D, 1).start()

        s0 = scores(0)
        if main:
            @pl.when(i + 2 * B < NS)
            def _():
                wq_part(i + 2 * B)
            wo_part(i + B)
        s1 = scores(1)
        o0 = values(0, [softmax(s) for s in s0])
        next_q(0)
        o1 = values(1, [softmax(s) for s in s1])
        oproj(0, o0)
        next_q(1)
        oproj(1, o1)
        tick()
        assert pos[0] == len(WTS) and bounds[-1] == len(sched)
        return carry

    assert len(TAIL_PRE) + 3 <= NSTAT < B
    lax.fori_loop(0, NS - B, functools.partial(step, main=True, static=False), 0)
    lax.fori_loop(NS - B, NS - NSTAT, functools.partial(step, main=False, static=False), 0)
    for u in range(NS - NSTAT, NS):
        step(u, 0, main=False, static=True)
    o_rect(0, (B - 1) * SQ, 0, 2 * D, 0).wait()
    o_rect((B - 1) * SQ, SQ, 0, 2 * D, 1).wait()


@jax.jit
def pallas_concat_heads__mha_block_cached__gqa_block_cached__near_ridge_kernel(
        A_x, A_k_cache, A_v_cache, A_wq, A_wo, B_x, B_k_cache, B_v_cache, B_wq, B_wo):
    def kv(a):
        return jnp.swapaxes(a, 2, 3).reshape(B * H * DH, SK)

    def tok(a):
        return a.reshape(B * SQ, D)

    any_spec = pl.BlockSpec(memory_space=pl.ANY)
    out = pl.pallas_call(
        _kernel,
        in_specs=[any_spec] * 10,
        out_specs=any_spec,
        out_shape=jax.ShapeDtypeStruct((B * SQ, 2 * D), BF16),
        scratch_shapes=[
            pltpu.VMEM((2, B * SQ, D), BF16),
            pltpu.VMEM((TOT, SK), BF16),
            pltpu.VMEM((B, 2, SQ, 512), BF16),
            pltpu.VMEM((B, SQ, 2 * D), F32),
            pltpu.VMEM((B * SQ, 2 * D), BF16),
            pltpu.SemaphoreType.DMA((2,)),
            pltpu.SemaphoreType.DMA((NB, 4)),
            pltpu.SemaphoreType.DMA((NW, 2)),
            pltpu.SemaphoreType.DMA((NW, 2)),
            pltpu.SemaphoreType.DMA((2,)),
        ],
        compiler_params=pltpu.CompilerParams(
            vmem_limit_bytes=64 * 1024 * 1024, disable_bounds_checks=True),
    )(tok(A_x), kv(A_k_cache), kv(A_v_cache), A_wq, A_wo,
      tok(B_x), kv(B_k_cache), kv(B_v_cache), B_wq, B_wo)
    return out.reshape(B, SQ, 2 * D)
```

```python
import functools
import math

import jax
import jax.numpy as jnp
from jax import lax
import jax.experimental.pallas as pl
import jax.experimental.pallas.tpu as pltpu

B, SQ, D = 8, 128, 640
H, SK, DH = 32, 1024, 192
F32 = jnp.float32
BF16 = jnp.bfloat16

HB = 2
NHG = H // HB
NS = NHG * B
W = HB * DH
R = HB * DH
NB = 4
NW = 4

WQ0 = NB * 4 * R
WO0 = WQ0 + NW * D
TOT = WO0 + NW * 2 * W

OFF = 13
STRIDE = 21
SHIFT = 26
TAIL_PRE = (10, 6, 3, 0)
PRE = 16
WTS = (0, 4, 3, 4, 4, 0, 6, 4, 0, 6, 4, 4, 6)
TWTS = (0, 4, 4, 4, 4, 0, 0, 6, 0, 6, 0, 4, 6)
XROWS = 32
OROWS, OSTREAMS = 16, 4


def _pieces():
    out = []
    rt, ct = divmod(OFF, 8)

    def clip(r0, nr, c0, nc):
        lo, hi = max(r0, 0), min(r0 + nr, R)
        return [(lo, hi - lo, c0, nc)] if hi > lo and nc > 0 else []

    for k in range(-1, R // 16):
        a = rt + 2 * k
        p = clip(a * 8, 16, ct * 128, SK - ct * 128) + clip((a + 1) * 8, 16, 0, ct * 128)
        if p:
            out.append(p)
    assert sum(nr * nc for p in out for (_, nr, _, nc) in p) == R * SK
    return out


_PCS = _pieces()
_NPC = len(_PCS)
assert math.gcd(STRIDE, _NPC) == 1
_ORDER = [(t * STRIDE) % _NPC for t in range(_NPC)]
_H1N = (_NPC + 1) // 2


def _pre_cnt(s):
    if s >= NS:
        return 0
    if s >= NS - len(TAIL_PRE):
        return TAIL_PRE[s - (NS - len(TAIL_PRE))]
    return _H1N


def _frame(s, generic=False):
    n0 = _H1N if generic else (_pre_cnt(s) if s >= 0 else _NPC)
    n1 = _H1N if generic else _pre_cnt(s + 1)
    own, nxt = _ORDER[n0:], _ORDER[:n1]
    groups, a, b = [], 0, 0
    while a < len(own) or b < len(nxt):
        if b < len(nxt) and (a >= len(own) or b * len(own) <= a * len(nxt)):
            groups.append((1, nxt[b]))
            b += 1
        else:
            groups.append((0, own[a]))
            a += 1
    return [(ds, [(j, _PCS[k]), (j + 1, _PCS[k])]) for (ds, k) in groups for j in (0, 2)]


def _sched(i_static):
    if i_static is None:
        f1 = f2 = _frame(0, generic=True)
    else:
        f1 = _frame(i_static + 1) if i_static + 1 < NS else []
        f2 = _frame(i_static + 2) if i_static + 2 < NS else []
    return [(1 + ds, p) for (ds, p) in f1[SHIFT:]] + [(2 + ds, p) for (ds, p) in f2[:SHIFT]]


def _bounds(ws, n):
    cum = [0]
    for w in ws:
        cum.append(cum[-1] + w)
    return [min(n, round(c * max(n, 40) / cum[-1])) for c in cum]


def _kernel(xa, ka, va, wqa, woa, xb, kb, vb, wqb, wob, o_hbm,
            x_buf, big, q_buf, acc_ref, o_buf,
            x_sem, kv_sem, wq_sem, wo_sem, o_sem):
    scale = (DH ** -0.5) * math.log2(math.e)
    kv_srcs = (ka, kb, va, vb)
    wq_srcs = (wqa, wqb)
    wo_srcs = (woa, wob)
    x_srcs = (xa, xb)

    def kv_base(i, j):
        return pl.multiple_of(((i % NB) * 4 + j) * R, 64)

    def kv_rect(i, j, r0, nr, c0, nc):
        row0 = pl.multiple_of(((i % B) * H + (i // B) * HB) * DH, 64)
        return pltpu.make_async_copy(
            kv_srcs[j].at[pl.ds(row0 + r0, nr), pl.ds(c0, nc)],
            big.at[pl.ds(kv_base(i, j) + r0, nr), pl.ds(c0, nc)],
            kv_sem.at[i % NB, j])

    def kv_pair(i, pair):
        for (j, piece) in pair:
            for rc in piece:
                kv_rect(i, j, *rc).start(priority=j % 2)

    def wq_base(hg):
        return pl.multiple_of(WQ0 + (hg % NW) * D, 64)

    def wo_base(hg, pi):
        return pl.multiple_of(WO0 + ((hg % NW) * 2 + pi) * W, 64)

    def wq_rows(hg, pi, r0, m):
        return pltpu.make_async_copy(
            wq_srcs[pi].at[pl.ds(r0, m), pl.ds(pl.multiple_of(hg * W, 128), W)],
            big.at[pl.ds(pl.multiple_of(wq_base(hg) + r0, 8), m), pl.ds(pi * W, W)],
            wq_sem.at[hg % NW, pi])

    def wo_rows(hg, pi, r0, m):
        return pltpu.make_async_copy(
            wo_srcs[pi].at[pl.ds(pl.multiple_of(hg * W + r0, 8), m), :],
            big.at[pl.ds(pl.multiple_of(wo_base(hg, pi) + r0, 8), m), pl.ds(0, D)],
            wo_sem.at[hg % NW, pi])

    def wq_part(g):
        m = D // (2 * B)
        for t in range(2):
            for pi in range(2):
                wq_rows(g // B, pi, pl.multiple_of(((g % B) * 2 + t) * m, 8), m).start(priority=pi)

    def wo_part(g):
        m = W // (2 * B)
        for t in range(2):
            for pi in range(2):
                wo_rows(g // B, pi, pl.multiple_of(((g % B) * 2 + t) * m, 8), m).start(priority=pi)

    def x_rows(pi, r0, m):
        return pltpu.make_async_copy(x_srcs[pi].at[pl.ds(r0, m)], x_buf.at[pi, pl.ds(r0, m)], x_sem.at[pi])

    def o_rect(r0, nr, c0, nc, k):
        return pltpu.make_async_copy(o_buf.at[pl.ds(r0, nr), pl.ds(c0, nc)],
                                     o_hbm.at[pl.ds(r0, nr), pl.ds(c0, nc)], o_sem.at[k])

    def loop(lo, hi, fn):
        def bd(t, c):
            fn(t)
            return c
        lax.fori_loop(lo, hi, bd, 0)

    lane = lax.broadcasted_iota(jnp.int32, (SQ, 128), 1)

    def qproj(hg, b, pi):
        x = x_buf[pi, pl.ds(pl.multiple_of(b * SQ, SQ), SQ), :]
        q = jnp.dot(x, big[pl.ds(wq_base(hg), D), pi * W:(pi + 1) * W],
                    preferred_element_type=F32) * scale
        qm = q[:, 128:256]
        q_buf[b, pi] = jnp.concatenate(
            [q[:, 0:128].astype(BF16),
             jnp.where(lane < 64, qm, 0.0).astype(BF16),
             jnp.where(lane >= 64, qm, 0.0).astype(BF16),
             q[:, 256:384].astype(BF16)], axis=1)

    def x_start(t):
        for pi in range(2):
            x_rows(pi, pl.multiple_of(t * XROWS, 8), XROWS).start(priority=pi)

    loop(0, B * SQ // XROWS, x_start)
    loop(0, B, wq_part)
    acc_ref[...] = jnp.zeros(acc_ref.shape, F32)
    work = [functools.partial(kv_pair, ds - 1, p) for (ds, p) in _frame(-1)]
    work += [functools.partial(kv_pair, ds, p) for (ds, p) in _frame(0)]
    work += [functools.partial(wo_part, g) for g in range(B)]
    work += [functools.partial(wq_part, g) for g in range(B, 2 * B)]
    work += [functools.partial(kv_pair, ds + 1, p) for (ds, p) in _frame(1)[:SHIFT]]
    for w in work[:PRE]:
        w()
    for pi in range(2):
        x_rows(pi, 0, B * SQ).wait()
    for pi in range(2):
        wq_rows(0, pi, 0, D).wait()
    rest = work[PRE:]
    for u in range(2 * B):
        for w in rest[(u * len(rest)) // (2 * B):((u + 1) * len(rest)) // (2 * B)]:
            w()
        qproj(0, u // 2, u % 2)

    def step(i, carry, main):
        hg = i // B
        b = i % B
        last = not main and i == NS - 1
        sched = _sched(None if main else i)
        bounds = _bounds(WTS if main else TWTS, len(sched))
        pos = [0]

        def tick():
            k = pos[0]
            pos[0] = k + 1
            for (la, p) in sched[bounds[k]:bounds[k + 1]]:
                kv_pair(i + la, p)

        if last:
            n = (B - 1) * SQ // OROWS
            h = -(-n // OSTREAMS)
            for k in [k for t in range(h) for k in range(t, n, h)]:
                o_rect(k * OROWS, OROWS, 0, 2 * D, 0).start()
        if main:
            @pl.when(b == 0)
            def _():
                for pi in range(2):
                    wq_rows(hg + 1, pi, 0, D).wait()
                for pi in range(2):
                    wo_rows(hg, pi, 0, W).wait()
        elif b == 0:
            for pi in range(2):
                wo_rows(hg, pi, 0, W).wait()
        for j in range(4):
            kv_rect(i, j, 0, R, 0, SK).wait()

        def next_q(pi):
            tick()
            if main:
                qproj(hg + 1, b, pi)

        def scores(pi):
            q = q_buf[b, pi]
            out = []
            for h in range(2):
                tick()
                out.append(jnp.dot(q[:, h * 256:(h + 1) * 256],
                                   big[pl.ds(kv_base(i, pi) + h * 128, 256), :],
                                   preferred_element_type=F32))
            return out

        def softmax(s):
            m = jnp.max(s, axis=-1, keepdims=True)
            p = jnp.exp2(s - m)
            return p.astype(BF16), jnp.sum(p, axis=-1, keepdims=True)

        def values(pi, ps):
            out = []
            for h in range(2):
                tick()
                p, l = ps[h]
                vt = big[pl.ds(kv_base(i, 2 + pi) + h * DH, DH), :]
                out.append((lax.dot_general(vt, p, (((1,), (1,)), ((), ())),
                                            preferred_element_type=F32), l))
            return out

        def oproj(pi, ots):
            tick()
            o = jnp.concatenate([t[0] for t in ots], axis=0).T
            r0 = 1.0 / ots[0][1]
            r1 = 1.0 / ots[1][1]
            o = jnp.concatenate([o[:, 0:128] * r0,
                                 o[:, 128:256] * jnp.where(lane < 64, r0, r1),
                                 o[:, 256:384] * r1], axis=1).astype(BF16)
            res = acc_ref[b, :, pi * D:(pi + 1) * D] + jnp.dot(
                o, big[pl.ds(wo_base(hg, pi), W), 0:D], preferred_element_type=F32)
            if main:
                acc_ref[b, :, pi * D:(pi + 1) * D] = res
            else:
                o_buf[pl.ds(pl.multiple_of(b * SQ, SQ), SQ), pi * D:(pi + 1) * D] = res.astype(BF16)
                if last:
                    o_rect((B - 1) * SQ, SQ, pi * D, D, 1).start()

        s0 = scores(0)
        if main:
            @pl.when(i + 2 * B < NS)
            def _():
                wq_part(i + 2 * B)
            wo_part(i + B)
        s1 = scores(1)
        o0 = values(0, [softmax(s) for s in s0])
        next_q(0)
        o1 = values(1, [softmax(s) for s in s1])
        oproj(0, o0)
        next_q(1)
        oproj(1, o1)
        tick()
        assert pos[0] == len(WTS) and bounds[-1] == len(sched)
        return carry

    assert len(TAIL_PRE) + 3 <= B
    lax.fori_loop(0, NS - B, functools.partial(step, main=True), 0)
    for u in range(NS - B, NS):
        step(u, 0, main=False)
    o_rect(0, (B - 1) * SQ, 0, 2 * D, 0).wait()
    o_rect((B - 1) * SQ, SQ, 0, 2 * D, 1).wait()


@jax.jit
def pallas_concat_heads__mha_block_cached__gqa_block_cached__near_ridge_kernel(
        A_x, A_k_cache, A_v_cache, A_wq, A_wo, B_x, B_k_cache, B_v_cache, B_wq, B_wo):
    def kv(a):
        return jnp.swapaxes(a, 2, 3).reshape(B * H * DH, SK)

    def tok(a):
        return a.reshape(B * SQ, D)

    any_spec = pl.BlockSpec(memory_space=pl.ANY)
    out = pl.pallas_call(
        _kernel,
        in_specs=[any_spec] * 10,
        out_specs=any_spec,
        out_shape=jax.ShapeDtypeStruct((B * SQ, 2 * D), BF16),
        scratch_shapes=[
            pltpu.VMEM((2, B * SQ, D), BF16),
            pltpu.VMEM((TOT, SK), BF16),
            pltpu.VMEM((B, 2, SQ, 512), BF16),
            pltpu.VMEM((B, SQ, 2 * D), F32),
            pltpu.VMEM((B * SQ, 2 * D), BF16),
            pltpu.SemaphoreType.DMA((2,)),
            pltpu.SemaphoreType.DMA((NB, 4)),
            pltpu.SemaphoreType.DMA((NW, 2)),
            pltpu.SemaphoreType.DMA((NW, 2)),
            pltpu.SemaphoreType.DMA((2,)),
        ],
        compiler_params=pltpu.CompilerParams(
            vmem_limit_bytes=64 * 1024 * 1024, disable_bounds_checks=True),
    )(tok(A_x), kv(A_k_cache), kv(A_v_cache), A_wq, A_wo,
      tok(B_x), kv(B_k_cache), kv(B_v_cache), B_wq, B_wo)
    return out.reshape(B, SQ, 2 * D)
```

```python
import functools
import math

import jax
import jax.numpy as jnp
from jax import lax
import jax.experimental.pallas as pl
import jax.experimental.pallas.tpu as pltpu

B, SQ, D = 8, 128, 640
H, SK, DH = 32, 1024, 192
F32 = jnp.float32
BF16 = jnp.bfloat16

HB = 2
NHG = H // HB
NS = NHG * B
W = HB * DH
NB = 4
NW = 4

KC = SK // 128
DC = D // 128
QC = H * DH // 128
QR = D // 8
BT = (W // 8) * KC
WOT = (W // 8) * DC
XT = (SQ // 8) * DC
PT = 16

WO0 = NB * 4 * BT
TOT = WO0 + 2 * NHG * WOT

OFF = 13
STRIDE = 21
SHIFT = 28
TAIL_PRE = (10, 6, 3, 0)
PRE = 24
QPRE = 36
WTS = (0, 5, 3, 4, 4, 3, 0, 6, 3, 4, 0, 7, 6)
TWTS = (0, 4, 4, 4, 4, 0, 0, 6, 0, 6, 0, 4, 6)
OROWS, OSTREAMS = 16, 4
SPL = 6


def _cuts(n):
    e = [0] + list(range(OFF, n, PT)) + [n]
    return [(a, z - a) for a, z in zip(e[:-1], e[1:])]


_PCS = _cuts(BT)
_NPC = len(_PCS)
assert math.gcd(STRIDE, _NPC) == 1
_ORDER = [(t * STRIDE) % _NPC for t in range(_NPC)]
_H1N = (_NPC + 1) // 2


def _mix(a, b):
    out, i, j = [], 0, 0
    while i < len(a) or j < len(b):
        if j < len(b) and (i >= len(a) or j * len(a) <= i * len(b)):
            out.append(b[j])
            j += 1
        else:
            out.append(a[i])
            i += 1
    return out


def _pre_cnt(s):
    if s >= NS:
        return 0
    if s >= NS - len(TAIL_PRE):
        return TAIL_PRE[s - (NS - len(TAIL_PRE))]
    return _H1N


def _frame(s, generic=False):
    n0 = _H1N if generic else (_pre_cnt(s) if s >= 0 else _NPC)
    n1 = _H1N if generic else _pre_cnt(s + 1)
    groups = _mix([(0, k) for k in _ORDER[n0:]], [(1, k) for k in _ORDER[:n1]])
    return [(ds, j, k) for (ds, k) in groups for j in (0, 2)]


def _sched(i_static):
    if i_static is None:
        f1 = f2 = _frame(0, generic=True)
    else:
        f1 = _frame(i_static + 1) if i_static + 1 < NS else []
        f2 = _frame(i_static + 2) if i_static + 2 < NS else []
    return ([(1 + ds, j, k) for (ds, j, k) in f1[SHIFT:]]
            + [(2 + ds, j, k) for (ds, j, k) in f2[:SHIFT]])


def _bounds(ws, n):
    cum = [0]
    for w in ws:
        cum.append(cum[-1] + w)
    return [min(n, round(c * max(n, 40) / cum[-1])) for c in cum]


def _untile(t, nc):
    r = t.shape[0] // nc
    t = t.reshape(r, nc, 8, 128)
    return jnp.concatenate([t[:, c].reshape(r * 8, 128) for c in range(nc)], axis=1)


def _kernel(xa, ka, va, wqa, woa, xb, kb, vb, wqb, wob, o_hbm,
            x_buf, big, wqr, q_buf, acc_ref, o_buf,
            x_sem, kv_sem, wq_sem, wo_sem, o_sem):
    scale = (DH ** -0.5) * math.log2(math.e)
    kv_srcs = (ka, kb, va, vb)
    wq_srcs = (wqa, wqb)
    wo_srcs = (woa, wob)
    x_srcs = (xa, xb)

    def kv_base(i, j):
        return ((i % NB) * 4 + j) * BT

    def kv_copy(i, j, t0, nt):
        src0 = ((i % B) * NHG + i // B) * BT
        return pltpu.make_async_copy(kv_srcs[j].at[pl.ds(src0 + t0, nt)],
                                     big.at[pl.ds(kv_base(i, j) + t0, nt)], kv_sem.at[i % NB, j])

    def kv_pair(i, j, k):
        t0, nt = _PCS[k]
        for u in range(2):
            kv_copy(i, j + u, t0, min(SPL, nt)).start(priority=u)
            if nt > SPL:
                kv_copy(i, j + u, t0 + SPL, nt - SPL).start(priority=u)

    def wo_copy(pi, t0, nt, s):
        return pltpu.make_async_copy(wo_srcs[pi].at[pl.ds(t0, nt)],
                                     big.at[pl.ds(WO0 + pi * NHG * WOT + t0, nt)], wo_sem.at[s, pi])

    def wo_piece(g, n):
        for pi in range(2):
            wo_copy(pi, g * WOT + OFF + n * PT, PT, g % NW).start(priority=pi)

    def wo_ends():
        return [wo_copy(pi, t0, nt, NW + e) for e, (t0, nt) in
                enumerate(((0, OFF), (NHG * WOT - PT + OFF, PT - OFF))) for pi in range(2)]

    def wo_wait(g, nt=WOT):
        for pi in range(2):
            wo_copy(pi, g * WOT + OFF, nt, g % NW).wait()

    def wq_tiles(pi, tr, c0, n, grp):
        return pltpu.make_async_copy(wq_srcs[pi].at[tr, pl.ds(c0, n)],
                                     wqr.at[pi, pl.ds(c0, n), pl.ds(pl.multiple_of(tr * 8, 8), 8)],
                                     wq_sem.at[grp, pi])

    def wq_a(t):
        for pi in range(2):
            wq_tiles(pi, (t + QR - 1) % QR, OFF + 2 * PT, PT - OFF, 3).start(priority=pi)
            wq_tiles(pi, t, 0, OFF, 0).start(priority=pi)

    def wq_bc(g):
        if isinstance(g, int):
            grp, tr = divmod(g, QR)
        else:
            grp = (g >= QR).astype(jnp.int32)
            tr = g - grp * QR
        tr = tr // 2 + (tr % 2) * (QR // 2)
        for pi in range(2):
            wq_tiles(pi, tr, OFF + PT * grp, PT, 1 + grp).start(priority=pi)

    def wq_wait(grp):
        c0, n = ((0, OFF), (OFF, PT), (OFF + PT, PT), (OFF + 2 * PT, PT - OFF))[grp]
        for pi in range(2):
            v = wqr.at[pi, pl.ds(c0, n)]
            pltpu.make_async_copy(v, v, wq_sem.at[grp, pi]).wait()

    def x_copy(pi, t0, nt, s):
        return pltpu.make_async_copy(x_srcs[pi].at[pl.ds(t0, nt)], x_buf.at[pi, pl.ds(t0, nt)],
                                     x_sem.at[pi, s])

    def o_rect(r0, nr, c0, nc, k):
        return pltpu.make_async_copy(o_buf.at[pl.ds(r0, nr), pl.ds(c0, nc)],
                                     o_hbm.at[pl.ds(r0, nr), pl.ds(c0, nc)], o_sem.at[k])

    def loop(lo, hi, fn):
        def bd(t, c):
            fn(t)
            return c
        lax.fori_loop(lo, hi, bd, 0)

    lane = lax.broadcasted_iota(jnp.int32, (SQ, 128), 1)

    def qproj(hg, b, pi):
        x = _untile(x_buf[pi, pl.ds(b * XT, XT)], DC)
        wq = jnp.concatenate([wqr[pi, hg * 3 + c] for c in range(3)], axis=1)
        q = jnp.dot(x, wq, preferred_element_type=F32)
        qm = q[:, 128:256]
        q_buf[b, pi] = jnp.concatenate(
            [q[:, 0:128].astype(BF16),
             jnp.where(lane < 64, qm, 0.0).astype(BF16),
             jnp.where(lane >= 64, qm, 0.0).astype(BF16),
             q[:, 256:384].astype(BF16)], axis=1)

    def x_wait(pi, g):
        lo = 0 if g == 0 else g * XT + OFF
        hi = min((g + 1) * XT + OFF, B * XT)
        x_copy(pi, lo, hi - lo, g).wait()

    for pi in range(2):
        x_copy(pi, 0, OFF, 0).start(priority=pi)
    for pi in range(2):
        x_copy(pi, B * XT - PT + OFF, PT - OFF, B - 1).start(priority=pi)

    def phase1(u):
        for v in range(4):
            wq_a(v * (QR // 4) + u)
            if v % 2 == 1:
                n = (v // 2) * (QR // 4) + u

                @pl.when(n < B * XT // PT - 1)
                def _():
                    for pi in range(2):
                        x_copy(pi, OFF + n * PT, PT, n // (XT // PT)).start(priority=pi)

    loop(0, QR // 4, phase1)
    acc_ref[...] = jnp.zeros(acc_ref.shape, F32)
    kvw = ([(ds - 1, j, k) for (ds, j, k) in _frame(-1)] + _frame(0)
           + [(ds + 1, j, k) for (ds, j, k) in _frame(1)[:SHIFT]])
    work = [functools.partial(kv_pair, *a) for a in kvw]
    for n, c in enumerate(wo_ends()):
        c.start(priority=n % 2)
    for w in work[:PRE]:
        w()
    wq_wait(0)
    wq_wait(3)
    rest = _mix(work[PRE:], [functools.partial(wo_piece, 0, n) for n in range(WOT // PT)])
    rest = _mix(rest, [functools.partial(wq_bc, g) for g in range(QPRE)])
    for u in range(2 * B):
        for w in rest[(u * len(rest)) // (2 * B):((u + 1) * len(rest)) // (2 * B)]:
            w()
        x_wait(u % 2, u // 2)
        qproj(0, u // 2, u % 2)
    for c in wo_ends():
        c.wait()

    def step(i, carry, main):
        hg = i // B
        b = i % B
        last = not main and i == NS - 1
        sched = _sched(None if main else i)
        bounds = _bounds(WTS if main else TWTS, len(sched))
        pos = [0]

        def tick():
            k = pos[0]
            pos[0] = k + 1
            for (la, j, p) in sched[bounds[k]:bounds[k + 1]]:
                kv_pair(i + la, j, p)

        if last:
            n = (B - 1) * SQ // OROWS
            h = -(-n // OSTREAMS)
            for k in [k for t in range(h) for k in range(t, n, h)]:
                o_rect(k * OROWS, OROWS, 0, 2 * D, 0).start()
        if main:
            @pl.when(b == 0)
            def _():
                for grp in (1, 2):
                    @pl.when(hg == (OFF + (grp - 1) * PT) // 3 - 1)
                    def _():
                        wq_wait(grp)
                wo_wait(hg)
        elif b == 0:
            wo_wait(hg, WOT - PT)
        for j in range(4):
            kv_copy(i, j, 0, BT).wait()

        def wo_next(u):
            if main:
                n = 2 * b + u

                @pl.when((n < WOT // PT) & (i * 2 + u < 2 * (NS - B) - 2))
                def _():
                    wo_piece(hg + 1, n)

        def next_q(pi):
            tick()
            if main:
                @pl.when(QPRE + i * 2 + pi < 2 * QR)
                def _():
                    wq_bc(QPRE + i * 2 + pi)
                qproj(hg + 1, b, pi)

        def scores(pi):
            out = []
            for h in range(2):
                tick()
                if h == 1:
                    wo_next(pi)
                kt = _untile(big[pl.ds(kv_base(i, pi) + h * 16 * KC, 32 * KC)], KC)
                out.append(jnp.dot(q_buf[b, pi, :, h * 256:(h + 1) * 256], kt,
                                   preferred_element_type=F32))
            return out

        def softmax(s):
            m = jnp.max(s, axis=-1, keepdims=True)
            p = jnp.exp2((s - m) * scale)
            return p.astype(BF16), jnp.sum(p, axis=-1, keepdims=True)

        def values(pi, ps):
            out = []
            for h in range(2):
                tick()
                p, l = ps[h]
                vt = _untile(big[pl.ds(kv_base(i, 2 + pi) + h * (BT // 2), BT // 2)], KC)
                out.append((lax.dot_general(vt, p, (((1,), (1,)), ((), ())),
                                            preferred_element_type=F32), l))
            return out

        def oproj(pi, ots):
            tick()
            o = jnp.concatenate([t[0] for t in ots], axis=0).T
            r0 = 1.0 / ots[0][1]
            r1 = 1.0 / ots[1][1]
            o = jnp.concatenate([o[:, 0:128] * r0,
                                 o[:, 128:256] * jnp.where(lane < 64, r0, r1),
                                 o[:, 256:384] * r1], axis=1).astype(BF16)
            wo = _untile(big[pl.ds(WO0 + (pi * NHG + hg) * WOT, WOT)], DC)
            res = acc_ref[b, :, pi * D:(pi + 1) * D] + jnp.dot(o, wo, preferred_element_type=F32)
            if main:
                acc_ref[b, :, pi * D:(pi + 1) * D] = res
            else:
                o_buf[pl.ds(b * SQ, SQ), pi * D:(pi + 1) * D] = res.astype(BF16)
                if last:
                    o_rect((B - 1) * SQ, SQ, pi * D, D, 1).start()

        s0 = scores(0)
        s1 = scores(1)
        o0 = values(0, [softmax(s) for s in s0])
        next_q(0)
        o1 = values(1, [softmax(s) for s in s1])
        oproj(0, o0)
        next_q(1)
        oproj(1, o1)
        tick()
        assert pos[0] == len(WTS) and bounds[-1] == len(sched)
        return carry

    assert len(TAIL_PRE) + 3 <= B
    lax.fori_loop(0, NS - B, functools.partial(step, main=True), 0)
    for u in range(NS - B, NS):
        step(u, 0, main=False)
    o_rect(0, (B - 1) * SQ, 0, 2 * D, 0).wait()
    o_rect((B - 1) * SQ, SQ, 0, 2 * D, 1).wait()


def _tiles(a):
    r, c = a.shape
    return a.reshape(r // 8, 8, c // 128, 128).transpose(0, 2, 1, 3)


@jax.jit
def pallas_concat_heads__mha_block_cached__gqa_block_cached__near_ridge_kernel(
        A_x, A_k_cache, A_v_cache, A_wq, A_wo, B_x, B_k_cache, B_v_cache, B_wq, B_wo):
    def flat(a):
        return _tiles(a).reshape(-1, 8, 128)

    def kv(a):
        return flat(jnp.swapaxes(a, 2, 3).reshape(B * H * DH, SK))

    def tok(a):
        return flat(a.reshape(B * SQ, D))

    any_spec = pl.BlockSpec(memory_space=pl.ANY)
    out = pl.pallas_call(
        _kernel,
        in_specs=[any_spec] * 10,
        out_specs=any_spec,
        out_shape=jax.ShapeDtypeStruct((B * SQ, 2 * D), BF16),
        scratch_shapes=[
            pltpu.VMEM((2, B * XT, 8, 128), BF16),
            pltpu.VMEM((TOT, 8, 128), BF16),
            pltpu.VMEM((2, QC, D, 128), BF16),
            pltpu.VMEM((B, 2, SQ, 512), BF16),
            pltpu.VMEM((B, SQ, 2 * D), F32),
            pltpu.VMEM((B * SQ, 2 * D), BF16),
            pltpu.SemaphoreType.DMA((2, B)),
            pltpu.SemaphoreType.DMA((NB, 4)),
            pltpu.SemaphoreType.DMA((4, 2)),
            pltpu.SemaphoreType.DMA((NW + 2, 2)),
            pltpu.SemaphoreType.DMA((2,)),
        ],
        compiler_params=pltpu.CompilerParams(
            vmem_limit_bytes=96 * 1024 * 1024, disable_bounds_checks=True),
    )(tok(A_x), kv(A_k_cache), kv(A_v_cache), _tiles(A_wq), flat(A_wo),
      tok(B_x), kv(B_k_cache), kv(B_v_cache), _tiles(B_wq), flat(B_wo))
    return out.reshape(B, SQ, 2 * D)
```

```python
import functools
import math

import jax
import jax.numpy as jnp
from jax import lax
import jax.experimental.pallas as pl
import jax.experimental.pallas.tpu as pltpu

B, SQ, D = 8, 128, 640
H, SK, DH = 32, 1024, 192
F32 = jnp.float32
BF16 = jnp.bfloat16

HB = 2
NHG = H // HB
NS = NHG * B
W = HB * DH
NB = 4
NW = 4

KC = SK // 128
DC = D // 128
QC = H * DH // 128
QR = D // 8
BT = (W // 8) * KC
WOT = (W // 8) * DC
XT = (SQ // 8) * DC
PT = 16

WO0 = NB * 4 * BT
TOT = WO0 + 2 * NHG * WOT

OFF = 13
STRIDE = 21
SHIFT = 27
TAIL_PRE = (10, 6, 3, 0)
PRE = 24
QPRE = 36
WTS = (4, 3, 4, 3, 4, 5, 0, 6, 4, 3, 0, 8, 4)
TWTS = (0, 4, 4, 4, 4, 0, 0, 6, 0, 6, 0, 4, 6)
OROWS, OSTREAMS = 16, 4
SPL = 6


def _cuts(n):
    e = [0] + list(range(OFF, n, PT)) + [n]
    return [(a, z - a) for a, z in zip(e[:-1], e[1:])]


_PCS = _cuts(BT)
_NPC = len(_PCS)
assert math.gcd(STRIDE, _NPC) == 1
_ORDER = [(t * STRIDE) % _NPC for t in range(_NPC)]
_H1N = (_NPC + 1) // 2


def _mix(a, b):
    out, i, j = [], 0, 0
    while i < len(a) or j < len(b):
        if j < len(b) and (i >= len(a) or j * len(a) <= i * len(b)):
            out.append(b[j])
            j += 1
        else:
            out.append(a[i])
            i += 1
    return out


def _pre_cnt(s):
    if s >= NS:
        return 0
    if s >= NS - len(TAIL_PRE):
        return TAIL_PRE[s - (NS - len(TAIL_PRE))]
    return _H1N


def _frame(s, generic=False):
    n0 = _H1N if generic else (_pre_cnt(s) if s >= 0 else _NPC)
    n1 = _H1N if generic else _pre_cnt(s + 1)
    groups = _mix([(0, k) for k in _ORDER[n0:]], [(1, k) for k in _ORDER[:n1]])
    return [(ds, j, k) for (ds, k) in groups for j in (0, 2)]


def _sched(i_static):
    if i_static is None:
        f1 = f2 = _frame(0, generic=True)
    else:
        f1 = _frame(i_static + 1) if i_static + 1 < NS else []
        f2 = _frame(i_static + 2) if i_static + 2 < NS else []
    return ([(1 + ds, j, k) for (ds, j, k) in f1[SHIFT:]]
            + [(2 + ds, j, k) for (ds, j, k) in f2[:SHIFT]])


def _bounds(ws, n):
    cum = [0]
    for w in ws:
        cum.append(cum[-1] + w)
    return [min(n, round(c * max(n, 40) / cum[-1])) for c in cum]


def _untile(t, nc):
    r = t.shape[0] // nc
    t = t.reshape(r, nc, 8, 128)
    return jnp.concatenate([t[:, c].reshape(r * 8, 128) for c in range(nc)], axis=1)


def _kernel(xa, ka, va, wqa, woa, xb, kb, vb, wqb, wob, o_hbm,
            x_buf, big, wqr, q_buf, acc_ref, o_buf,
            x_sem, kv_sem, wq_sem, wo_sem, o_sem):
    scale = (DH ** -0.5) * math.log2(math.e)
    kv_srcs = (ka, kb, va, vb)
    wq_srcs = (wqa, wqb)
    wo_srcs = (woa, wob)
    x_srcs = (xa, xb)

    def kv_base(i, j):
        return ((i % NB) * 4 + j) * BT

    def kv_copy(i, j, t0, nt):
        src0 = ((i % B) * NHG + i // B) * BT
        return pltpu.make_async_copy(kv_srcs[j].at[pl.ds(src0 + t0, nt)],
                                     big.at[pl.ds(kv_base(i, j) + t0, nt)], kv_sem.at[i % NB, j])

    def kv_pair(i, j, k):
        t0, nt = _PCS[k]
        for u in range(2):
            kv_copy(i, j + u, t0, min(SPL, nt)).start(priority=u)
            if nt > SPL:
                kv_copy(i, j + u, t0 + SPL, nt - SPL).start(priority=u)

    def wo_copy(pi, t0, nt, s):
        return pltpu.make_async_copy(wo_srcs[pi].at[pl.ds(t0, nt)],
                                     big.at[pl.ds(WO0 + pi * NHG * WOT + t0, nt)], wo_sem.at[s, pi])

    def wo_piece(g, n):
        for pi in range(2):
            wo_copy(pi, g * WOT + OFF + n * PT, PT, g % NW).start(priority=pi)

    def wo_ends():
        return [wo_copy(pi, t0, nt, NW + e) for e, (t0, nt) in
                enumerate(((0, OFF), (NHG * WOT - PT + OFF, PT - OFF))) for pi in range(2)]

    def wo_wait(g, nt=WOT):
        for pi in range(2):
            wo_copy(pi, g * WOT + OFF, nt, g % NW).wait()

    def wq_tiles(pi, tr, c0, n, grp):
        return pltpu.make_async_copy(wq_srcs[pi].at[tr, pl.ds(c0, n)],
                                     wqr.at[pi, pl.ds(c0, n), tr],
                                     wq_sem.at[grp, pi])

    def wq_a(t):
        for pi in range(2):
            wq_tiles(pi, (t + QR - 1) % QR, OFF + 2 * PT, PT - OFF, 3).start(priority=pi)
            wq_tiles(pi, t, 0, OFF, 0).start(priority=pi)

    def wq_bc(g):
        if isinstance(g, int):
            grp, tr = divmod(g, QR)
        else:
            grp = (g >= QR).astype(jnp.int32)
            tr = g - grp * QR
        tr = tr // 2 + (tr % 2) * (QR // 2)
        for pi in range(2):
            wq_tiles(pi, tr, OFF + PT * grp, PT, 1 + grp).start(priority=pi)

    def wq_wait(grp):
        c0, n = ((0, OFF), (OFF, PT), (OFF + PT, PT), (OFF + 2 * PT, PT - OFF))[grp]
        for pi in range(2):
            v = wqr.at[pi, pl.ds(c0, n)]
            pltpu.make_async_copy(v, v, wq_sem.at[grp, pi]).wait()

    def x_copy(pi, t0, nt, s):
        return pltpu.make_async_copy(x_srcs[pi].at[pl.ds(t0, nt)], x_buf.at[pi, pl.ds(t0, nt)],
                                     x_sem.at[pi, s])

    def o_rect(r0, nr, c0, nc, k):
        return pltpu.make_async_copy(o_buf.at[pl.ds(r0, nr), pl.ds(c0, nc)],
                                     o_hbm.at[pl.ds(r0, nr), pl.ds(c0, nc)], o_sem.at[k])

    def loop(lo, hi, fn):
        def bd(t, c):
            fn(t)
            return c
        lax.fori_loop(lo, hi, bd, 0)

    lane = lax.broadcasted_iota(jnp.int32, (SQ, 128), 1)

    def qproj(hg, b, pi):
        x = _untile(x_buf[pi, pl.ds(b * XT, XT)], DC)
        wq = jnp.concatenate([wqr[pi, hg * 3 + c].reshape(D, 128) for c in range(3)], axis=1)
        q = jnp.dot(x, wq, preferred_element_type=F32)
        qm = q[:, 128:256]
        q_buf[b, pi] = jnp.concatenate(
            [q[:, 0:128].astype(BF16),
             jnp.where(lane < 64, qm, 0.0).astype(BF16),
             jnp.where(lane >= 64, qm, 0.0).astype(BF16),
             q[:, 256:384].astype(BF16)], axis=1)

    def x_wait(pi, g):
        lo = 0 if g == 0 else g * XT + OFF
        hi = min((g + 1) * XT + OFF, B * XT)
        x_copy(pi, lo, hi - lo, g).wait()

    for pi in range(2):
        x_copy(pi, 0, OFF, 0).start(priority=pi)
    for pi in range(2):
        x_copy(pi, B * XT - PT + OFF, PT - OFF, B - 1).start(priority=pi)

    def phase1(u):
        for v in range(4):
            wq_a(v * (QR // 4) + u)
            if v % 2 == 1:
                n = (v // 2) * (QR // 4) + u

                @pl.when(n < B * XT // PT - 1)
                def _():
                    for pi in range(2):
                        x_copy(pi, OFF + n * PT, PT, n // (XT // PT)).start(priority=pi)

    loop(0, QR // 4, phase1)
    acc_ref[...] = jnp.zeros(acc_ref.shape, F32)
    kvw = ([(ds - 1, j, k) for (ds, j, k) in _frame(-1)] + _frame(0)
           + [(ds + 1, j, k) for (ds, j, k) in _frame(1)[:SHIFT]])
    work = [functools.partial(kv_pair, *a) for a in kvw]
    for n, c in enumerate(wo_ends()):
        c.start(priority=n % 2)
    for w in work[:PRE]:
        w()
    wq_wait(0)
    wq_wait(3)
    rest = _mix(work[PRE:], [functools.partial(wo_piece, 0, n) for n in range(WOT // PT)])
    rest = _mix(rest, [functools.partial(wq_bc, g) for g in range(QPRE)])
    for u in range(2 * B):
        for w in rest[(u * len(rest)) // (2 * B):((u + 1) * len(rest)) // (2 * B)]:
            w()
        x_wait(u % 2, u // 2)
        qproj(0, u // 2, u % 2)
    for c in wo_ends():
        c.wait()

    def step(i, carry, main):
        hg = i // B
        b = i % B
        last = not main and i == NS - 1
        sched = _sched(None if main else i)
        bounds = _bounds(WTS if main else TWTS, len(sched))
        pos = [0]

        def tick():
            k = pos[0]
            pos[0] = k + 1
            for (la, j, p) in sched[bounds[k]:bounds[k + 1]]:
                kv_pair(i + la, j, p)

        if last:
            n = (B - 1) * SQ // OROWS
            h = -(-n // OSTREAMS)
            for k in [k for t in range(h) for k in range(t, n, h)]:
                o_rect(k * OROWS, OROWS, 0, 2 * D, 0).start()
        if main:
            @pl.when(b == 0)
            def _():
                for grp in (1, 2):
                    @pl.when(hg == (OFF + (grp - 1) * PT) // 3 - 1)
                    def _():
                        wq_wait(grp)
                wo_wait(hg)
        elif b == 0:
            wo_wait(hg, WOT - PT)
        for j in range(4):
            kv_copy(i, j, 0, BT).wait()

        def wo_next(u):
            if main:
                n = 2 * b + u

                @pl.when((n < WOT // PT) & (i * 2 + u < 2 * (NS - B) - 2))
                def _():
                    wo_piece(hg + 1, n)

        def next_q(pi):
            tick()
            if main:
                @pl.when(QPRE + i * 2 + pi < 2 * QR)
                def _():
                    wq_bc(QPRE + i * 2 + pi)
                qproj(hg + 1, b, pi)

        def scores(pi):
            out = []
            for h in range(2):
                tick()
                if h == 1:
                    wo_next(pi)
                kt = _untile(big[pl.ds(kv_base(i, pi) + h * 16 * KC, 32 * KC)], KC)
                out.append(jnp.dot(q_buf[b, pi, :, h * 256:(h + 1) * 256], kt,
                                   preferred_element_type=F32))
            return out

        def softmax(s):
            m = jnp.max(s, axis=-1, keepdims=True)
            p = jnp.exp2((s - m) * scale)
            return p.astype(BF16), jnp.sum(p, axis=-1, keepdims=True)

        def values(pi, ps):
            out = []
            for h in range(2):
                tick()
                p, l = ps[h]
                vt = _untile(big[pl.ds(kv_base(i, 2 + pi) + h * (BT // 2), BT // 2)], KC)
                out.append((lax.dot_general(vt, p, (((1,), (1,)), ((), ())),
                                            preferred_element_type=F32), l))
            return out

        def oproj(pi, ots):
            tick()
            o = jnp.concatenate([t[0] for t in ots], axis=0).T
            r0 = 1.0 / ots[0][1]
            r1 = 1.0 / ots[1][1]
            o = jnp.concatenate([o[:, 0:128] * r0,
                                 o[:, 128:256] * jnp.where(lane < 64, r0, r1),
                                 o[:, 256:384] * r1], axis=1).astype(BF16)
            wo = _untile(big[pl.ds(WO0 + (pi * NHG + hg) * WOT, WOT)], DC)
            res = acc_ref[b, :, pi * D:(pi + 1) * D] + jnp.dot(o, wo, preferred_element_type=F32)
            if main:
                acc_ref[b, :, pi * D:(pi + 1) * D] = res
            else:
                o_buf[pl.ds(b * SQ, SQ), pi * D:(pi + 1) * D] = res.astype(BF16)
                if last:
                    o_rect((B - 1) * SQ, SQ, pi * D, D, 1).start()

        s0 = scores(0)
        s1 = scores(1)
        o0 = values(0, [softmax(s) for s in s0])
        next_q(0)
        o1 = values(1, [softmax(s) for s in s1])
        oproj(0, o0)
        next_q(1)
        oproj(1, o1)
        tick()
        assert pos[0] == len(WTS) and bounds[-1] == len(sched)
        return carry

    assert len(TAIL_PRE) + 3 <= B
    lax.fori_loop(0, NS - B, functools.partial(step, main=True), 0)
    for u in range(NS - B, NS):
        step(u, 0, main=False)
    o_rect(0, (B - 1) * SQ, 0, 2 * D, 0).wait()
    o_rect((B - 1) * SQ, SQ, 0, 2 * D, 1).wait()


def _tiles(a):
    r, c = a.shape
    return a.reshape(r // 8, 8, c // 128, 128).transpose(0, 2, 1, 3)


@jax.jit
def pallas_concat_heads__mha_block_cached__gqa_block_cached__near_ridge_kernel(
        A_x, A_k_cache, A_v_cache, A_wq, A_wo, B_x, B_k_cache, B_v_cache, B_wq, B_wo):
    def flat(a):
        return _tiles(a).reshape(-1, 8, 128)

    def kv(a):
        return flat(jnp.swapaxes(a, 2, 3).reshape(B * H * DH, SK))

    def tok(a):
        return flat(a.reshape(B * SQ, D))

    any_spec = pl.BlockSpec(memory_space=pl.ANY)
    out = pl.pallas_call(
        _kernel,
        in_specs=[any_spec] * 10,
        out_specs=any_spec,
        out_shape=jax.ShapeDtypeStruct((B * SQ, 2 * D), BF16),
        scratch_shapes=[
            pltpu.VMEM((2, B * XT, 8, 128), BF16),
            pltpu.VMEM((TOT, 8, 128), BF16),
            pltpu.VMEM((2, QC, QR, 8, 128), BF16),
            pltpu.VMEM((B, 2, SQ, 512), BF16),
            pltpu.VMEM((B, SQ, 2 * D), F32),
            pltpu.VMEM((B * SQ, 2 * D), BF16),
            pltpu.SemaphoreType.DMA((2, B)),
            pltpu.SemaphoreType.DMA((NB, 4)),
            pltpu.SemaphoreType.DMA((4, 2)),
            pltpu.SemaphoreType.DMA((NW + 2, 2)),
            pltpu.SemaphoreType.DMA((2,)),
        ],
        compiler_params=pltpu.CompilerParams(
            vmem_limit_bytes=96 * 1024 * 1024, disable_bounds_checks=True),
    )(tok(A_x), kv(A_k_cache), kv(A_v_cache), _tiles(A_wq), flat(A_wo),
      tok(B_x), kv(B_k_cache), kv(B_v_cache), _tiles(B_wq), flat(B_wo))
    return out.reshape(B, SQ, 2 * D)
```

```python
import functools
import math

import jax
import jax.numpy as jnp
from jax import lax
import jax.experimental.pallas as pl
import jax.experimental.pallas.tpu as pltpu

B, SQ, D = 8, 128, 640
H, SK, DH = 32, 1024, 192
F32 = jnp.float32
BF16 = jnp.bfloat16

HB = 2
NHG = H // HB
NS = NHG * B
W = HB * DH
NB = 4
NW = 2

KC = SK // 128
DC = D // 128
QC = H * DH // 128
QR = D // 8
BT = (W // 8) * KC
WOT = (W // 8) * DC
XT = (SQ // 8) * DC
PT = 16

WO0 = NB * 4 * BT
TOT = WO0 + 2 * NHG * WOT

OFF = 13
STRIDE = 21
SHIFT = 27
TAIL_PRE = (10, 6, 3, 0)
PRE = 24
QPRE = 36
WTS = (4, 3, 4, 3, 4, 5, 0, 6, 4, 3, 0, 8, 4)
TWTS = (0, 4, 4, 4, 4, 0, 0, 6, 0, 6, 0, 4, 6)
OROWS, OSTREAMS = 16, 4
SPL = 6


def _cuts(n):
    e = [0] + list(range(OFF, n, PT)) + [n]
    return [(a, z - a) for a, z in zip(e[:-1], e[1:])]


_PCS = _cuts(BT)
_NPC = len(_PCS)
assert math.gcd(STRIDE, _NPC) == 1
_ORDER = [(t * STRIDE) % _NPC for t in range(_NPC)]
_H1N = (_NPC + 1) // 2


def _mix(a, b):
    out, i, j = [], 0, 0
    while i < len(a) or j < len(b):
        if j < len(b) and (i >= len(a) or j * len(a) <= i * len(b)):
            out.append(b[j])
            j += 1
        else:
            out.append(a[i])
            i += 1
    return out


def _pre_cnt(s):
    if s >= NS:
        return 0
    if s >= NS - len(TAIL_PRE):
        return TAIL_PRE[s - (NS - len(TAIL_PRE))]
    return _H1N


def _frame(s, generic=False):
    n0 = _H1N if generic else (_pre_cnt(s) if s >= 0 else _NPC)
    n1 = _H1N if generic else _pre_cnt(s + 1)
    groups = _mix([(0, k) for k in _ORDER[n0:]], [(1, k) for k in _ORDER[:n1]])
    return [(ds, j, k) for (ds, k) in groups for j in (0, 2)]


def _sched(i_static):
    if i_static is None:
        f1 = f2 = _frame(0, generic=True)
    else:
        f1 = _frame(i_static + 1) if i_static + 1 < NS else []
        f2 = _frame(i_static + 2) if i_static + 2 < NS else []
    return ([(1 + ds, j, k) for (ds, j, k) in f1[SHIFT:]]
            + [(2 + ds, j, k) for (ds, j, k) in f2[:SHIFT]])


def _bounds(ws, n):
    cum = [0]
    for w in ws:
        cum.append(cum[-1] + w)
    return [min(n, round(c * max(n, 40) / cum[-1])) for c in cum]


def _untile(t, nc):
    r = t.shape[0] // nc
    t = t.reshape(r, nc, 8, 128)
    return jnp.concatenate([t[:, c].reshape(r * 8, 128) for c in range(nc)], axis=1)


def _kernel(xa, ka, va, wqa, woa, xb, kb, vb, wqb, wob, o_hbm,
            x_buf, big, wqr, q_buf, acc_ref, o_buf,
            x_sem, kv_sem, wq_sem, wo_sem, o_sem):
    scale = (DH ** -0.5) * math.log2(math.e)
    kv_srcs = (ka, kb, va, vb)
    wq_srcs = (wqa, wqb)
    wo_srcs = (woa, wob)
    x_srcs = (xa, xb)

    def kv_base(i, j):
        return ((i % NB) * 4 + j) * BT

    def kv_copy(i, j, t0, nt):
        src0 = ((i % B) * NHG + i // B) * BT
        return pltpu.make_async_copy(kv_srcs[j].at[pl.ds(src0 + t0, nt)],
                                     big.at[pl.ds(kv_base(i, j) + t0, nt)], kv_sem.at[i % NB])

    def kv_pair(i, j, k):
        t0, nt = _PCS[k]
        for u in range(2):
            kv_copy(i, j + u, t0, min(SPL, nt)).start(priority=u)
            if nt > SPL:
                kv_copy(i, j + u, t0 + SPL, nt - SPL).start(priority=u)

    def wo_copy(pi, t0, nt, s):
        return pltpu.make_async_copy(wo_srcs[pi].at[pl.ds(t0, nt)],
                                     big.at[pl.ds(WO0 + pi * NHG * WOT + t0, nt)], wo_sem.at[s, pi])

    def wo_piece(g, n):
        for pi in range(2):
            wo_copy(pi, g * WOT + OFF + n * PT, PT, g % NW).start(priority=pi)

    def wo_ends():
        return [wo_copy(pi, t0, nt, NW + e) for e, (t0, nt) in
                enumerate(((0, OFF), (NHG * WOT - PT + OFF, PT - OFF))) for pi in range(2)]

    def wo_wait(g, nt=WOT):
        for pi in range(2):
            wo_copy(pi, g * WOT + OFF, nt, g % NW).wait()

    def wq_tiles(pi, tr, c0, n, grp):
        return pltpu.make_async_copy(wq_srcs[pi].at[tr, pl.ds(c0, n)],
                                     wqr.at[pi, pl.ds(c0, n), tr],
                                     wq_sem.at[grp])

    def wq_a(t):
        for pi in range(2):
            wq_tiles(pi, jnp.where(t == 0, QR - 1, t - 1), OFF + 2 * PT, PT - OFF, 3).start(priority=pi)
            wq_tiles(pi, t, 0, OFF, 0).start(priority=pi)

    def wq_bc(g):
        if isinstance(g, int):
            grp, tr = divmod(g, QR)
        else:
            grp = (g >= QR).astype(jnp.int32)
            tr = g - grp * QR
        tr = tr // 2 + (tr % 2) * (QR // 2)
        for pi in range(2):
            wq_tiles(pi, tr, OFF + PT * grp, PT, 1 + grp).start(priority=pi)

    def wq_wait(grp):
        c0, n = ((0, OFF), (OFF, PT), (OFF + PT, PT), (OFF + 2 * PT, PT - OFF))[grp]
        v = wqr.at[:, pl.ds(c0, n)]
        pltpu.make_async_copy(v, v, wq_sem.at[grp]).wait()

    def x_copy(pi, t0, nt, s):
        return pltpu.make_async_copy(x_srcs[pi].at[pl.ds(t0, nt)], x_buf.at[pi, pl.ds(t0, nt)],
                                     x_sem.at[pi, s])

    def o_rect(r0, nr, c0, nc, k):
        return pltpu.make_async_copy(o_buf.at[pl.ds(r0, nr), pl.ds(c0, nc)],
                                     o_hbm.at[pl.ds(r0, nr), pl.ds(c0, nc)], o_sem.at[k])

    def loop(lo, hi, fn):
        def bd(t, c):
            fn(t)
            return c
        lax.fori_loop(lo, hi, bd, 0)

    lane = lax.broadcasted_iota(jnp.int32, (SQ, 128), 1)

    def qproj(hg, b, pi):
        x = _untile(x_buf[pi, pl.ds(b * XT, XT)], DC)
        wq = jnp.concatenate([wqr[pi, hg * 3 + c].reshape(D, 128) for c in range(3)], axis=1)
        q = jnp.dot(x, wq, preferred_element_type=F32)
        qm = q[:, 128:256]
        q_buf[b, pi] = jnp.concatenate(
            [q[:, 0:128].astype(BF16),
             jnp.where(lane < 64, qm, 0.0).astype(BF16),
             jnp.where(lane >= 64, qm, 0.0).astype(BF16),
             q[:, 256:384].astype(BF16)], axis=1)

    def x_wait(pi, g):
        lo = 0 if g == 0 else g * XT + OFF
        hi = min((g + 1) * XT + OFF, B * XT)
        x_copy(pi, lo, hi - lo, g).wait()

    for pi in range(2):
        x_copy(pi, 0, OFF, 0).start(priority=pi)
    for pi in range(2):
        x_copy(pi, B * XT - PT + OFF, PT - OFF, B - 1).start(priority=pi)

    assert all((n * 13) >> 6 == n // (XT // PT) for n in range(B * XT // PT))

    def phase1(u):
        for v in range(4):
            wq_a(v * (QR // 4) + u)
            if v % 2 == 1:
                n = (v // 2) * (QR // 4) + u

                @pl.when(n < B * XT // PT - 1)
                def _():
                    for pi in range(2):
                        x_copy(pi, OFF + n * PT, PT, (n * 13) >> 6).start(priority=pi)

    loop(0, QR // 4, phase1)
    acc_ref[...] = jnp.zeros(acc_ref.shape, F32)
    kvw = ([(ds - 1, j, k) for (ds, j, k) in _frame(-1)] + _frame(0)
           + [(ds + 1, j, k) for (ds, j, k) in _frame(1)[:SHIFT]])
    work = [functools.partial(kv_pair, *a) for a in kvw]
    for n, c in enumerate(wo_ends()):
        c.start(priority=n % 2)
    for w in work[:PRE]:
        w()
    wq_wait(0)
    wq_wait(3)
    rest = _mix(work[PRE:], [functools.partial(wo_piece, 0, n) for n in range(WOT // PT)])
    rest = _mix(rest, [functools.partial(wq_bc, g) for g in range(QPRE)])
    for u in range(2 * B):
        for w in rest[(u * len(rest)) // (2 * B):((u + 1) * len(rest)) // (2 * B)]:
            w()
        x_wait(u % 2, u // 2)
        qproj(0, u // 2, u % 2)
    for c in wo_ends():
        c.wait()

    def step(i, carry, main):
        hg = i // B
        b = i % B
        last = not main and i == NS - 1
        sched = _sched(None if main else i)
        bounds = _bounds(WTS if main else TWTS, len(sched))
        pos = [0]

        def tick():
            k = pos[0]
            pos[0] = k + 1
            for (la, j, p) in sched[bounds[k]:bounds[k + 1]]:
                kv_pair(i + la, j, p)

        if last:
            n = (B - 1) * SQ // OROWS
            h = -(-n // OSTREAMS)
            for k in [k for t in range(h) for k in range(t, n, h)]:
                o_rect(k * OROWS, OROWS, 0, 2 * D, 0).start()
        if main:
            @pl.when(b == 0)
            def _():
                for grp in (1, 2):
                    @pl.when(hg == (OFF + (grp - 1) * PT) // 3 - 1)
                    def _():
                        wq_wait(grp)
                wo_wait(hg)
        elif b == 0:
            wo_wait(hg, WOT - PT)
        slot = big.at[pl.ds(kv_base(i, 0), 4 * BT)]
        pltpu.make_async_copy(slot, slot, kv_sem.at[i % NB]).wait()

        def wo_next(u):
            if main:
                n = 2 * b + u

                @pl.when((n < WOT // PT) & (i * 2 + u < 2 * (NS - B) - 2))
                def _():
                    wo_piece(hg + 1, n)

        def next_q(pi):
            tick()
            if main:
                @pl.when(QPRE + i * 2 + pi < 2 * QR)
                def _():
                    wq_bc(QPRE + i * 2 + pi)
                qproj(hg + 1, b, pi)

        def scores(pi):
            out = []
            for h in range(2):
                tick()
                if h == 1:
                    wo_next(pi)
                kt = _untile(big[pl.ds(kv_base(i, pi) + h * 16 * KC, 32 * KC)], KC)
                out.append(jnp.dot(q_buf[b, pi, :, h * 256:(h + 1) * 256], kt,
                                   preferred_element_type=F32))
            return out

        def softmax(s):
            m = jnp.max(s, axis=-1, keepdims=True)
            p = jnp.exp2((s - m) * scale)
            return p.astype(BF16), jnp.sum(p, axis=-1, keepdims=True)

        def values(pi, ps):
            out = []
            for h in range(2):
                tick()
                p, l = ps[h]
                vt = _untile(big[pl.ds(kv_base(i, 2 + pi) + h * (BT // 2), BT // 2)], KC)
                out.append((lax.dot_general(vt, p, (((1,), (1,)), ((), ())),
                                            preferred_element_type=F32), l))
            return out

        def oproj(pi, ots):
            tick()
            o = jnp.concatenate([t[0] for t in ots], axis=0).T
            r0 = 1.0 / ots[0][1]
            r1 = 1.0 / ots[1][1]
            o = jnp.concatenate([o[:, 0:128] * r0,
                                 o[:, 128:256] * jnp.where(lane < 64, r0, r1),
                                 o[:, 256:384] * r1], axis=1).astype(BF16)
            wo = _untile(big[pl.ds(WO0 + (pi * NHG + hg) * WOT, WOT)], DC)
            res = acc_ref[b, :, pi * D:(pi + 1) * D] + jnp.dot(o, wo, preferred_element_type=F32)
            if main:
                acc_ref[b, :, pi * D:(pi + 1) * D] = res
            else:
                o_buf[pl.ds(b * SQ, SQ), pi * D:(pi + 1) * D] = res.astype(BF16)
                if last:
                    o_rect((B - 1) * SQ, SQ, pi * D, D, 1).start()

        s0 = scores(0)
        s1 = scores(1)
        o0 = values(0, [softmax(s) for s in s0])
        next_q(0)
        o1 = values(1, [softmax(s) for s in s1])
        oproj(0, o0)
        next_q(1)
        oproj(1, o1)
        tick()
        assert pos[0] == len(WTS) and bounds[-1] == len(sched)
        return carry

    assert len(TAIL_PRE) + 3 <= B
    lax.fori_loop(0, NS - B, functools.partial(step, main=True), 0)
    for u in range(NS - B, NS):
        step(u, 0, main=False)
    o_rect(0, (B - 1) * SQ, 0, 2 * D, 0).wait()
    o_rect((B - 1) * SQ, SQ, 0, 2 * D, 1).wait()


def _tiles(a):
    r, c = a.shape
    return a.reshape(r // 8, 8, c // 128, 128).transpose(0, 2, 1, 3)


def _compiler_params():
    kw = dict(vmem_limit_bytes=96 * 1024 * 1024, disable_bounds_checks=True)
    try:
        return pltpu.CompilerParams(disable_semaphore_checks=True, **kw)
    except TypeError:
        return pltpu.CompilerParams(**kw)


@jax.jit
def pallas_concat_heads__mha_block_cached__gqa_block_cached__near_ridge_kernel(
        A_x, A_k_cache, A_v_cache, A_wq, A_wo, B_x, B_k_cache, B_v_cache, B_wq, B_wo):
    def flat(a):
        return _tiles(a).reshape(-1, 8, 128)

    def kv(a):
        return flat(jnp.swapaxes(a, 2, 3).reshape(B * H * DH, SK))

    def tok(a):
        return flat(a.reshape(B * SQ, D))

    any_spec = pl.BlockSpec(memory_space=pl.ANY)
    out = pl.pallas_call(
        _kernel,
        in_specs=[any_spec] * 10,
        out_specs=any_spec,
        out_shape=jax.ShapeDtypeStruct((B * SQ, 2 * D), BF16),
        scratch_shapes=[
            pltpu.VMEM((2, B * XT, 8, 128), BF16),
            pltpu.VMEM((TOT, 8, 128), BF16),
            pltpu.VMEM((2, QC, QR, 8, 128), BF16),
            pltpu.VMEM((B, 2, SQ, 512), BF16),
            pltpu.VMEM((B, SQ, 2 * D), F32),
            pltpu.VMEM((B * SQ, 2 * D), BF16),
            pltpu.SemaphoreType.DMA((2, B)),
            pltpu.SemaphoreType.DMA((NB,)),
            pltpu.SemaphoreType.DMA((4,)),
            pltpu.SemaphoreType.DMA((NW + 2, 2)),
            pltpu.SemaphoreType.DMA((2,)),
        ],
        compiler_params=_compiler_params(),
    )(tok(A_x), kv(A_k_cache), kv(A_v_cache), _tiles(A_wq), flat(A_wo),
      tok(B_x), kv(B_k_cache), kv(B_v_cache), _tiles(B_wq), flat(B_wo))
    return out.reshape(B, SQ, 2 * D)
```

```python
import functools
import math

import jax
import jax.numpy as jnp
from jax import lax
import jax.experimental.pallas as pl
import jax.experimental.pallas.tpu as pltpu

B, SQ, D = 8, 128, 640
H, SK, DH = 32, 1024, 192
F32 = jnp.float32
BF16 = jnp.bfloat16

HB = 2
NHG = H // HB
NS = NHG * B
W = HB * DH
NB = 4
NW = 2

KC = SK // 128
DC = D // 128
QC = H * DH // 128
QR = D // 8
BT = (W // 8) * KC
WOT = (W // 8) * DC
XT = (SQ // 8) * DC
PT = 16

WO0 = NB * 4 * BT
TOT = WO0 + 2 * NHG * WOT

OFF = 13
STRIDE = 21
SHIFT = 27
TAIL_PRE = (10, 6, 3, 0)
PRE = 24
QPRE = 36
WTS = (4, 3, 4, 3, 4, 5, 0, 6, 4, 3, 0, 8, 4)
TWTS = (0, 4, 4, 4, 4, 0, 0, 6, 0, 6, 0, 4, 6)
OROWS, OSTREAMS = 16, 4
SPL = 2


def _cuts(n):
    e = [0] + list(range(OFF, n, PT)) + [n]
    return [(a, z - a) for a, z in zip(e[:-1], e[1:])]


_PCS = _cuts(BT)
_NPC = len(_PCS)
assert math.gcd(STRIDE, _NPC) == 1
_ORDER = [(t * STRIDE) % _NPC for t in range(_NPC)]
_H1N = (_NPC + 1) // 2


def _mix(a, b):
    out, i, j = [], 0, 0
    while i < len(a) or j < len(b):
        if j < len(b) and (i >= len(a) or j * len(a) <= i * len(b)):
            out.append(b[j])
            j += 1
        else:
            out.append(a[i])
            i += 1
    return out


def _pre_cnt(s):
    if s >= NS:
        return 0
    if s >= NS - len(TAIL_PRE):
        return TAIL_PRE[s - (NS - len(TAIL_PRE))]
    return _H1N


def _frame(s, generic=False):
    n0 = _H1N if generic else (_pre_cnt(s) if s >= 0 else _NPC)
    n1 = _H1N if generic else _pre_cnt(s + 1)
    groups = _mix([(0, k) for k in _ORDER[n0:]], [(1, k) for k in _ORDER[:n1]])
    return [(ds, j, k) for (ds, k) in groups for j in (0, 2)]


def _sched(i_static):
    if i_static is None:
        f1 = f2 = _frame(0, generic=True)
    else:
        f1 = _frame(i_static + 1) if i_static + 1 < NS else []
        f2 = _frame(i_static + 2) if i_static + 2 < NS else []
    return ([(1 + ds, j, k) for (ds, j, k) in f1[SHIFT:]]
            + [(2 + ds, j, k) for (ds, j, k) in f2[:SHIFT]])


def _bounds(ws, n):
    cum = [0]
    for w in ws:
        cum.append(cum[-1] + w)
    return [min(n, round(c * max(n, 40) / cum[-1])) for c in cum]


def _untile(t, nc):
    r = t.shape[0] // nc
    t = t.reshape(r, nc, 8, 128)
    return jnp.concatenate([t[:, c].reshape(r * 8, 128) for c in range(nc)], axis=1)


def _kernel(xa, ka, va, wqa, woa, xb, kb, vb, wqb, wob, o_hbm,
            x_buf, big, wqr, q_buf, acc_ref, o_buf,
            x_sem, kv_sem, wq_sem, wo_sem, o_sem):
    scale = (DH ** -0.5) * math.log2(math.e)
    kv_srcs = (ka, kb, va, vb)
    wq_srcs = (wqa, wqb)
    wo_srcs = (woa, wob)
    x_srcs = (xa, xb)

    def kv_base(i, j):
        return ((i % NB) * 4 + j) * BT

    def kv_copy(i, j, t0, nt):
        src0 = ((i % B) * NHG + i // B) * BT
        return pltpu.make_async_copy(kv_srcs[j].at[pl.ds(src0 + t0, nt)],
                                     big.at[pl.ds(kv_base(i, j) + t0, nt)], kv_sem.at[i % NB])

    def kv_pair(i, j, k):
        t0, nt = _PCS[k]
        kv_copy(i, j, t0, nt).start(priority=0)
        kv_copy(i, j + 1, t0, min(SPL, nt)).start(priority=1)
        if nt > SPL:
            kv_copy(i, j + 1, t0 + SPL, nt - SPL).start(priority=1)

    def wo_copy(pi, t0, nt, s):
        return pltpu.make_async_copy(wo_srcs[pi].at[pl.ds(t0, nt)],
                                     big.at[pl.ds(WO0 + pi * NHG * WOT + t0, nt)], wo_sem.at[s, pi])

    def wo_piece(g, n):
        for pi in range(2):
            wo_copy(pi, g * WOT + OFF + n * PT, PT, g % NW).start(priority=pi)

    def wo_ends():
        return [wo_copy(pi, t0, nt, NW + e) for e, (t0, nt) in
                enumerate(((0, OFF), (NHG * WOT - PT + OFF, PT - OFF))) for pi in range(2)]

    def wo_wait(g, nt=WOT):
        for pi in range(2):
            wo_copy(pi, g * WOT + OFF, nt, g % NW).wait()

    def wq_tiles(pi, tr, c0, n, grp):
        return pltpu.make_async_copy(wq_srcs[pi].at[tr, pl.ds(c0, n)],
                                     wqr.at[pi, pl.ds(c0, n), tr],
                                     wq_sem.at[grp])

    def wq_a(t):
        for pi in range(2):
            wq_tiles(pi, jnp.where(t == 0, QR - 1, t - 1), OFF + 2 * PT, PT - OFF, 3).start(priority=pi)
            wq_tiles(pi, t, 0, OFF, 0).start(priority=pi)

    def wq_bc(g):
        if isinstance(g, int):
            grp, tr = divmod(g, QR)
        else:
            grp = (g >= QR).astype(jnp.int32)
            tr = g - grp * QR
        tr = tr // 2 + (tr % 2) * (QR // 2)
        for pi in range(2):
            wq_tiles(pi, tr, OFF + PT * grp, PT, 1 + grp).start(priority=pi)

    def wq_wait(grp):
        c0, n = ((0, OFF), (OFF, PT), (OFF + PT, PT), (OFF + 2 * PT, PT - OFF))[grp]
        v = wqr.at[:, pl.ds(c0, n)]
        pltpu.make_async_copy(v, v, wq_sem.at[grp]).wait()

    def x_copy(pi, t0, nt, s):
        return pltpu.make_async_copy(x_srcs[pi].at[pl.ds(t0, nt)], x_buf.at[pi, pl.ds(t0, nt)],
                                     x_sem.at[pi, s])

    def o_rect(r0, nr, c0, nc, k):
        return pltpu.make_async_copy(o_buf.at[pl.ds(r0, nr), pl.ds(c0, nc)],
                                     o_hbm.at[pl.ds(r0, nr), pl.ds(c0, nc)], o_sem.at[k])

    def loop(lo, hi, fn):
        def bd(t, c):
            fn(t)
            return c
        lax.fori_loop(lo, hi, bd, 0)

    lane = lax.broadcasted_iota(jnp.int32, (SQ, 128), 1)

    def qproj(hg, b, pi):
        x = _untile(x_buf[pi, pl.ds(b * XT, XT)], DC)
        wq = jnp.concatenate([wqr[pi, hg * 3 + c].reshape(D, 128) for c in range(3)], axis=1)
        q = jnp.dot(x, wq, preferred_element_type=F32)
        qm = q[:, 128:256]
        q_buf[b, pi] = jnp.concatenate(
            [q[:, 0:128].astype(BF16),
             jnp.where(lane < 64, qm, 0.0).astype(BF16),
             jnp.where(lane >= 64, qm, 0.0).astype(BF16),
             q[:, 256:384].astype(BF16)], axis=1)

    def x_wait(pi, g):
        lo = 0 if g == 0 else g * XT + OFF
        hi = min((g + 1) * XT + OFF, B * XT)
        x_copy(pi, lo, hi - lo, g).wait()

    for pi in range(2):
        x_copy(pi, 0, OFF, 0).start(priority=pi)
    for pi in range(2):
        x_copy(pi, B * XT - PT + OFF, PT - OFF, B - 1).start(priority=pi)

    assert all((n * 13) >> 6 == n // (XT // PT) for n in range(B * XT // PT))

    def phase1(u):
        for v in range(4):
            wq_a(v * (QR // 4) + u)
            if v % 2 == 1:
                n = (v // 2) * (QR // 4) + u

                @pl.when(n < B * XT // PT - 1)
                def _():
                    for pi in range(2):
                        x_copy(pi, OFF + n * PT, PT, (n * 13) >> 6).start(priority=pi)

    loop(0, QR // 4, phase1)
    acc_ref[...] = jnp.zeros(acc_ref.shape, F32)
    kvw = ([(ds - 1, j, k) for (ds, j, k) in _frame(-1)] + _frame(0)
           + [(ds + 1, j, k) for (ds, j, k) in _frame(1)[:SHIFT]])
    work = [functools.partial(kv_pair, *a) for a in kvw]
    for n, c in enumerate(wo_ends()):
        c.start(priority=n % 2)
    for w in work[:PRE]:
        w()
    wq_wait(0)
    wq_wait(3)
    rest = _mix(work[PRE:], [functools.partial(wo_piece, 0, n) for n in range(WOT // PT)])
    rest = _mix(rest, [functools.partial(wq_bc, g) for g in range(QPRE)])
    for u in range(2 * B):
        for w in rest[(u * len(rest)) // (2 * B):((u + 1) * len(rest)) // (2 * B)]:
            w()
        x_wait(u % 2, u // 2)
        qproj(0, u // 2, u % 2)
    for c in wo_ends():
        c.wait()

    def step(i, carry, main):
        hg = i // B
        b = i % B
        last = not main and i == NS - 1
        sched = _sched(None if main else i)
        bounds = _bounds(WTS if main else TWTS, len(sched))
        pos = [0]

        def tick():
            k = pos[0]
            pos[0] = k + 1
            for (la, j, p) in sched[bounds[k]:bounds[k + 1]]:
                kv_pair(i + la, j, p)

        if last:
            n = (B - 1) * SQ // OROWS
            h = -(-n // OSTREAMS)
            for k in [k for t in range(h) for k in range(t, n, h)]:
                o_rect(k * OROWS, OROWS, 0, 2 * D, 0).start()
        if main:
            @pl.when(b == 0)
            def _():
                for grp in (1, 2):
                    @pl.when(hg == (OFF + (grp - 1) * PT) // 3 - 1)
                    def _():
                        wq_wait(grp)
                wo_wait(hg)
        elif b == 0:
            wo_wait(hg, WOT - PT)
        slot = big.at[pl.ds(kv_base(i, 0), 4 * BT)]
        pltpu.make_async_copy(slot, slot, kv_sem.at[i % NB]).wait()

        def wo_next(u):
            if main:
                n = 2 * b + u

                @pl.when((n < WOT // PT) & (i * 2 + u < 2 * (NS - B) - 2))
                def _():
                    wo_piece(hg + 1, n)

        def next_q(pi):
            tick()
            if main:
                @pl.when(QPRE + i * 2 + pi < 2 * QR)
                def _():
                    wq_bc(QPRE + i * 2 + pi)
                qproj(hg + 1, b, pi)

        def scores(pi):
            out = []
            for h in range(2):
                tick()
                if h == 1:
                    wo_next(pi)
                kt = _untile(big[pl.ds(kv_base(i, pi) + h * 16 * KC, 32 * KC)], KC)
                out.append(jnp.dot(q_buf[b, pi, :, h * 256:(h + 1) * 256], kt,
                                   preferred_element_type=F32))
            return out

        def softmax(s):
            m = jnp.max(s, axis=-1, keepdims=True)
            p = jnp.exp2((s - m) * scale)
            return p.astype(BF16), jnp.sum(p, axis=-1, keepdims=True)

        def values(pi, ps):
            out = []
            for h in range(2):
                tick()
                p, l = ps[h]
                vt = _untile(big[pl.ds(kv_base(i, 2 + pi) + h * (BT // 2), BT // 2)], KC)
                out.append((lax.dot_general(vt, p, (((1,), (1,)), ((), ())),
                                            preferred_element_type=F32), l))
            return out

        def oproj(pi, ots):
            tick()
            o = jnp.concatenate([t[0] for t in ots], axis=0).T
            r0 = 1.0 / ots[0][1]
            r1 = 1.0 / ots[1][1]
            o = jnp.concatenate([o[:, 0:128] * r0,
                                 o[:, 128:256] * jnp.where(lane < 64, r0, r1),
                                 o[:, 256:384] * r1], axis=1).astype(BF16)
            wo = _untile(big[pl.ds(WO0 + (pi * NHG + hg) * WOT, WOT)], DC)
            res = acc_ref[b, :, pi * D:(pi + 1) * D] + jnp.dot(o, wo, preferred_element_type=F32)
            if main:
                acc_ref[b, :, pi * D:(pi + 1) * D] = res
            else:
                o_buf[pl.ds(b * SQ, SQ), pi * D:(pi + 1) * D] = res.astype(BF16)
                if last:
                    o_rect((B - 1) * SQ, SQ, pi * D, D, 1).start()

        s0 = scores(0)
        s1 = scores(1)
        o0 = values(0, [softmax(s) for s in s0])
        next_q(0)
        o1 = values(1, [softmax(s) for s in s1])
        oproj(0, o0)
        next_q(1)
        oproj(1, o1)
        tick()
        assert pos[0] == len(WTS) and bounds[-1] == len(sched)
        return carry

    assert len(TAIL_PRE) + 3 <= B
    lax.fori_loop(0, NS - B, functools.partial(step, main=True), 0)
    for u in range(NS - B, NS):
        step(u, 0, main=False)
    o_rect(0, (B - 1) * SQ, 0, 2 * D, 0).wait()
    o_rect((B - 1) * SQ, SQ, 0, 2 * D, 1).wait()


def _tiles(a):
    r, c = a.shape
    return a.reshape(r // 8, 8, c // 128, 128).transpose(0, 2, 1, 3)


def _compiler_params():
    kw = dict(vmem_limit_bytes=96 * 1024 * 1024, disable_bounds_checks=True)
    try:
        return pltpu.CompilerParams(disable_semaphore_checks=True, **kw)
    except TypeError:
        return pltpu.CompilerParams(**kw)


@jax.jit
def pallas_concat_heads__mha_block_cached__gqa_block_cached__near_ridge_kernel(
        A_x, A_k_cache, A_v_cache, A_wq, A_wo, B_x, B_k_cache, B_v_cache, B_wq, B_wo):
    def flat(a):
        return _tiles(a).reshape(-1, 8, 128)

    def kv(a):
        return flat(jnp.swapaxes(a, 2, 3).reshape(B * H * DH, SK))

    def tok(a):
        return flat(a.reshape(B * SQ, D))

    any_spec = pl.BlockSpec(memory_space=pl.ANY)
    out = pl.pallas_call(
        _kernel,
        in_specs=[any_spec] * 10,
        out_specs=any_spec,
        out_shape=jax.ShapeDtypeStruct((B * SQ, 2 * D), BF16),
        scratch_shapes=[
            pltpu.VMEM((2, B * XT, 8, 128), BF16),
            pltpu.VMEM((TOT, 8, 128), BF16),
            pltpu.VMEM((2, QC, QR, 8, 128), BF16),
            pltpu.VMEM((B, 2, SQ, 512), BF16),
            pltpu.VMEM((B, SQ, 2 * D), F32),
            pltpu.VMEM((B * SQ, 2 * D), BF16),
            pltpu.SemaphoreType.DMA((2, B)),
            pltpu.SemaphoreType.DMA((NB,)),
            pltpu.SemaphoreType.DMA((4,)),
            pltpu.SemaphoreType.DMA((NW + 2, 2)),
            pltpu.SemaphoreType.DMA((2,)),
        ],
        compiler_params=_compiler_params(),
    )(tok(A_x), kv(A_k_cache), kv(A_v_cache), _tiles(A_wq), flat(A_wo),
      tok(B_x), kv(B_k_cache), kv(B_v_cache), _tiles(B_wq), flat(B_wo))
    return out.reshape(B, SQ, 2 * D)
```
